```python
import jax
import jax.numpy as jnp

def _softmax(x, axis=-1):
    return jax.nn.softmax(x, axis=axis)

def _gelu(x):
    return jax.nn.gelu(x, approximate=True)

def _silu(x):
    return jax.nn.silu(x)

def _sigmoid(x):
    return jax.nn.sigmoid(x)

def _layernorm(x, axis=-1, eps=1e-05):
    m = jnp.mean(x, axis=axis, keepdims=True)
    v = jnp.var(x, axis=axis, keepdims=True)
    return (x - m) / jnp.sqrt(v + eps)

def _scatter_add(tgt, idx, src, axis=0):
    return tgt.at[idx].add(src)

def _segment_sum(src, seg, n):
    return jax.ops.segment_sum(src, seg, n)

class _Rng:

    def __init__(self, key):
        self._k = key

    def _next(self):
        self._k, sub = jax.random.split(self._k)
        return sub

    def normal(self, shape):
        return jax.random.normal(self._next(), shape, dtype=jnp.bfloat16)

    def randint(self, lo, hi, shape):
        return jax.random.randint(self._next(), shape, lo, hi, dtype=jnp.int32)

    def uniform(self, shape, lo=0.0, hi=1.0):
        return jax.random.uniform(self._next(), shape, jnp.bfloat16, lo, hi)

    def permutation(self, n):
        return jax.random.permutation(self._next(), n)
kernel_name = 'interleave_layers__memory_aug_recurrent_mem_tr__mixer_s_mlp__prompt'

def setup_inputs():
    _rng = _Rng(jax.random.key(int.from_bytes(__import__("os").urandom(4), "little")))
    _w = lambda a: (lambda t: t.astype(jnp.bfloat16) if jnp.issubdtype(t.dtype, jnp.floating) else t)(jnp.asarray(a))

    def _A_setup():
        B, S, Dm = (1, 2048, 640)
        H, Dh = (32, 192)
        M, seg = (8, 32)
        seg = min(seg, S)
        S = S // seg * seg
        return {'x': _w((lambda *s: _rng.normal(s) * 0.05)(B, S, Dm)), 'mem0': _w((lambda *s: _rng.normal(s) * 0.05)(B, M, Dm)), 'Wq': _w((lambda *s: _rng.normal(s) * 0.05)(Dm, H, Dh) * Dm ** (-0.5)), 'Wk': _w((lambda *s: _rng.normal(s) * 0.05)(Dm, H, Dh) * Dm ** (-0.5)), 'Wv': _w((lambda *s: _rng.normal(s) * 0.05)(Dm, H, Dh) * Dm ** (-0.5)), 'Wo': _w((lambda *s: _rng.normal(s) * 0.05)(H, Dh, Dm) * (H * Dh) ** (-0.5)), 'seg_len': seg}
    _A_in = _A_setup()

    def _B_setup():
        B, S, D, F = (1, 2048, 640, 1536)
        return {'x': _w((lambda *s: _rng.normal(s) * 0.05)(B, S, D)), 'w1': _w((lambda *s: _rng.normal(s) * 0.05)(D, D) * D ** (-0.5)), 'w2': _w((lambda *s: _rng.normal(s) * 0.05)(D, D) * D ** (-0.5)), 'w3': _w((lambda *s: _rng.normal(s) * 0.05)(D, F) * D ** (-0.5)), 'w4': _w((lambda *s: _rng.normal(s) * 0.05)(F, D) * F ** (-0.5))}
    _B_in = _B_setup()
    return {'A_x': _A_in['x'], 'A_mem0': _A_in['mem0'], 'A_Wq': _A_in['Wq'], 'A_Wk': _A_in['Wk'], 'A_Wv': _A_in['Wv'], 'A_Wo': _A_in['Wo'], 'A_seg_len': _A_in['seg_len'], 'B_x': _B_in['x'], 'B_w1': _B_in['w1'], 'B_w2': _B_in['w2'], 'B_w3': _B_in['w3'], 'B_w4': _B_in['w4']}

def reference(A_x, A_mem0, A_Wq, A_Wk, A_Wv, A_Wo, A_seg_len, B_x, B_w1, B_w2, B_w3, B_w4):

    def _A_ref(x, mem0, Wq, Wk, Wv, Wo, seg_len):
        B, S, Dm = x.shape
        H, Dh = (Wq.shape[1], Wq.shape[2])
        M = mem0.shape[1]
        scale = Dh ** (-0.5)
        n_seg = S // seg_len
        L = M + seg_len
        idx = jnp.arange(L)
        mask = (idx[:, None] < M) | (idx[:, None] >= idx[None, :])
        mem = mem0
        outs = []
        for s in range(n_seg):
            xs = x[:, s * seg_len:(s + 1) * seg_len, :].copy()
            h = jnp.concatenate([mem, xs], axis=1)
            q = jnp.einsum('btd,dhe->bhte', h, Wq)
            k = jnp.einsum('btd,dhe->bhte', h, Wk)
            v = jnp.einsum('btd,dhe->bhte', h, Wv)
            scores = jnp.einsum('bhqe,bhke->bhqk', q, k) * scale
            scores = jnp.where(mask[None, None], scores, -1000000000.0)
            p = _softmax(scores, axis=-1)
            o = jnp.einsum('bhqk,bhke->bhqe', p, v)
            o = jnp.einsum('bhte,hed->btd', o, Wo)
            mem = o[:, :M, :].copy()
            outs.append(o[:, M:, :])
        return jnp.concatenate(outs, axis=1)

    def _B_ref(x, w1, w2, w3, w4):
        B, S, D = x.shape
        h = _gelu(_layernorm(x, axis=-1) @ w1)
        c = D // 4
        g0 = jnp.pad(h[:, :, 0 * c:1 * c], ((0, 0), (1, 0), (0, 0)))[:, :S, :]
        g1 = jnp.pad(h[:, :, 1 * c:2 * c], ((0, 0), (0, 1), (0, 0)))[:, 1:, :]
        g2 = jnp.pad(h[:, :, 2 * c:3 * c], ((0, 0), (2, 0), (0, 0)))[:, :S, :]
        g3 = jnp.pad(h[:, :, 3 * c:], ((0, 0), (0, 2), (0, 0)))[:, 2:, :]
        hs = jnp.concatenate([g0, g1, g2, g3], axis=-1) @ w2
        x1 = x + hs
        h2 = _gelu(_layernorm(x1, axis=-1) @ w3) @ w4
        return x1 + h2
    x = A_x
    x = x + _A_ref(_layernorm(x, axis=-1), A_mem0, A_Wq, A_Wk, A_Wv, A_Wo, A_seg_len)
    x = x + _B_ref(_layernorm(x, axis=-1), B_w1, B_w2, B_w3, B_w4)
    x = x + _A_ref(_layernorm(x, axis=-1), A_mem0, A_Wq, A_Wk, A_Wv, A_Wo, A_seg_len)
    x = x + _B_ref(_layernorm(x, axis=-1), B_w1, B_w2, B_w3, B_w4)
    return x
```

```python
import functools

import jax
import jax.numpy as jnp
from jax import lax
import jax.experimental.pallas as pl
import jax.experimental.pallas.tpu as pltpu

BF = jnp.bfloat16
F32 = jnp.float32
I32 = jnp.int32

S, D, H, E, M, SEG, F = 2048, 640, 32, 192, 8, 32, 1536
L = M + SEG
NSEG = S // SEG
NP = H // 2
PW = 2 * E
SCALE = float(E ** -0.5)
EPS = 1e-5
RB = 128
PAD = 8
GROUP = D // 4
LAGS = (1, 4, 5)


def _ln(x):
    m = jnp.mean(x, axis=-1, keepdims=True)
    c = x - m
    v = jnp.mean(c * c, axis=-1, keepdims=True)
    return c * lax.rsqrt(v + EPS)


def _gelu(x):
    k = 0.7978845608028654
    return 0.5 * x * (1.0 + jnp.tanh(k * (x + 0.044715 * (x * x * x))))


def _dot(a, b):
    return jnp.dot(a, b, preferred_element_type=F32)


def _unpack(w):
    return pltpu.bitcast(w, BF)


def _a_step(h, wq, wk, wv, wo):
    lane = lax.broadcasted_iota(I32, (L, 128), 1)
    lo = lane < 64
    col = lax.broadcasted_iota(I32, (L, 2 * L), 1)
    row = lax.broadcasted_iota(I32, (L, 2 * L), 0)
    first = col < L
    key = jnp.where(first, col, col - L)
    allowed = (row < M) | (row >= key)
    zt = jnp.zeros((L, 128), F32)
    q_, k_, v_, p_, o_ = {}, {}, {}, {}, {}
    acc = [None]

    def blockdiag(t):
        t0, t1, t2 = t[:, 0:128], t[:, 128:256], t[:, 256:384]
        top = jnp.concatenate([t0, jnp.where(lo, t1, 0.0), zt], axis=1)
        bot = jnp.concatenate([zt, jnp.where(lo, 0.0, t1), t2], axis=1)
        return jnp.concatenate([top, bot], axis=0).astype(BF)

    def qkv(p):
        q_[p] = _dot(h, _unpack(wq[p]))
        k_[p] = blockdiag(_dot(h, _unpack(wk[p])))
        v_[p] = blockdiag(_dot(h, _unpack(wv[p])))

    def qk(p):
        s = lax.dot_general(q_.pop(p), k_.pop(p), (((1,), (1,)), ((), ())),
                            preferred_element_type=F32)
        s = jnp.where(allowed, s * SCALE, -1e9)
        m1 = jnp.max(jnp.where(first, s, -jnp.inf), axis=1, keepdims=True)
        m2 = jnp.max(jnp.where(first, -jnp.inf, s), axis=1, keepdims=True)
        e = jnp.exp(s - jnp.where(first, m1, m2))
        l1 = jnp.sum(jnp.where(first, e, 0.0), axis=1, keepdims=True)
        l2 = jnp.sum(jnp.where(first, 0.0, e), axis=1, keepdims=True)
        p_[p] = e * pl.reciprocal(jnp.where(first, l1, l2), approx=False)

    def pv(p):
        o_[p] = _dot(p_.pop(p), v_.pop(p))

    def out(p):
        y = _dot(o_.pop(p), _unpack(wo[p]))
        acc[0] = y if acc[0] is None else acc[0] + y

    la, lb, lc = LAGS
    for t in range(NP + lc):
        if t < NP:
            qkv(t)
        if 0 <= t - la < NP:
            qk(t - la)
        if 0 <= t - lb < NP:
            pv(t - lb)
        if 0 <= t - lc < NP:
            out(t - lc)
    return acc[0]


def _shift_gather(hbuf, r0, rows):
    lane = lax.broadcasted_iota(I32, (rows, 128), 1)
    shifts = (-1, 1, -2, 2)
    tiles = []
    for t in range(D // 128):
        g_lo = (t * 128) // GROUP
        g_hi = (t * 128 + 127) // GROUP
        a = hbuf[t, pl.ds(r0 + PAD + shifts[g_lo], rows), :]
        if g_hi != g_lo:
            b = hbuf[t, pl.ds(r0 + PAD + shifts[g_hi], rows), :]
            a = jnp.where(lane < (g_hi * GROUP - t * 128), a, b)
        tiles.append(a)
    return jnp.concatenate(tiles, axis=1)


def _kernel(x_hbm, mem_hbm, wq_hbm, wk_hbm, wv_hbm, wo_hbm, w1_hbm, w2_hbm, w3_hbm, w4_hbm,
            o_hbm,
            xb, memb, sq, sk, sv, so, s1, s2, s3, s4,
            wq, wk, wv, wo, w1, w2, w3, w4,
            xres, xn, hbuf, ob, sem_x, sem_w, sem_b, sem_o):
    def x_copy():
        return pltpu.make_async_copy(x_hbm, xb, sem_x.at[0])

    def mem_copy():
        return pltpu.make_async_copy(mem_hbm, memb, sem_x.at[1])

    def w_copy(i, p):
        src, dst = ((wq_hbm, sq), (wk_hbm, sk), (wv_hbm, sv), (wo_hbm, so))[i]
        sl = pl.ds(p * PW, PW)
        return pltpu.make_async_copy(src.at[sl, :], dst.at[sl, :], sem_w.at[i, p])

    def b_copy(i):
        src, dst = ((w1_hbm, s1), (w2_hbm, s2), (w3_hbm, s3), (w4_hbm, s4))[i]
        return pltpu.make_async_copy(src, dst, sem_b.at[i])

    x_copy().start()
    mem_copy().start()
    for p in range(NP):
        for i in range(4):
            w_copy(i, p).start()
    for i in range(4):
        b_copy(i).start()

    hbuf[:, pl.ds(0, PAD), :] = jnp.zeros((D // 128, PAD, 128), F32)
    hbuf[:, pl.ds(PAD + S, PAD), :] = jnp.zeros((D // 128, PAD, 128), F32)

    x_copy().wait()
    mem_copy().wait()

    def init_rows(i, c):
        r0 = pl.multiple_of(i * RB, RB)
        x = xb[pl.ds(r0, RB), :].astype(F32)
        xres[pl.ds(r0, RB), :] = x
        xn[pl.ds(r0, RB), :] = _ln(x)
        return c
    lax.fori_loop(0, S // RB, init_rows, 0)

    def prep_pair(p, c):
        r0 = pl.multiple_of(p * PW, PW)
        for i, (src, dst) in enumerate(((sq, wq), (sk, wk), (sv, wv))):
            pltpu.make_async_copy(src.at[pl.ds(r0, PW), :], src.at[pl.ds(r0, PW), :],
                                  sem_w.at[i, p]).wait()
            dst[p] = pltpu.bitcast(src[pl.ds(r0, PW), :].T, I32)
        pltpu.make_async_copy(so.at[pl.ds(r0, PW), :], so.at[pl.ds(r0, PW), :],
                              sem_w.at[3, p]).wait()
        wo[p] = pltpu.bitcast(so[pl.ds(r0, PW), :], I32)
        return c
    lax.fori_loop(0, NP, prep_pair, 0)

    for i, (src, dst) in enumerate(((s1, w1), (s2, w2), (s3, w3), (s4, w4))):
        b_copy(i).wait()
        dst[...] = pltpu.bitcast(src[...], I32)

    def out_copy(i):
        sl = pl.ds(pl.multiple_of(i * RB, RB), RB)
        return pltpu.make_async_copy(ob.at[sl, :], o_hbm.at[sl, :], sem_o.at[i])

    def layer(l, c):
        def seg_step(s, mem):
            r0 = pl.multiple_of(s * SEG, SEG)
            h = jnp.concatenate([mem, xn[pl.ds(r0, SEG), :]], axis=0)
            o = _a_step(h, wq, wk, wv, wo)
            xres[pl.ds(r0, SEG), :] = xres[pl.ds(r0, SEG), :] + o[M:, :]
            return o[:M, :]
        lax.fori_loop(0, NSEG, seg_step, memb[...].astype(F32))

        def b1(i, c2):
            r0 = pl.multiple_of(i * RB, RB)
            xin = _ln(xres[pl.ds(r0, RB), :])
            xn[pl.ds(r0, RB), :] = xin
            hh = _gelu(_dot(_ln(xin), _unpack(w1[...])))
            for t in range(D // 128):
                hbuf[t, pl.ds(r0 + PAD, RB), :] = hh[:, t * 128:(t + 1) * 128]
            return c2
        lax.fori_loop(0, S // RB, b1, 0)

        def b2(i, c2):
            r0 = pl.multiple_of(i * RB, RB)
            g = _shift_gather(hbuf, r0, RB)
            x1 = xn[pl.ds(r0, RB), :] + _dot(g, _unpack(w2[...]))
            u = _gelu(_dot(_ln(x1), _unpack(w3[...])))
            xo = xres[pl.ds(r0, RB), :] + (x1 + _dot(u, _unpack(w4[...])))
            xres[pl.ds(r0, RB), :] = xo
            xn[pl.ds(r0, RB), :] = _ln(xo)
            ob[pl.ds(r0, RB), :] = xo.astype(BF)

            @pl.when(l == 1)
            def _():
                out_copy(i).start()
            return c2
        lax.fori_loop(0, S // RB, b2, 0)
        return c
    lax.fori_loop(0, 2, layer, 0)

    for i in range(S // RB):
        out_copy(i).wait()


@jax.jit
def _impl(A_x, A_mem0, A_Wq, A_Wk, A_Wv, A_Wo, B_w1, B_w2, B_w3, B_w4):
    x = A_x.reshape(S, D)
    mem0 = A_mem0.reshape(M, D)
    wqt = jnp.transpose(A_Wq, (1, 2, 0)).reshape(H * E, D)
    wkt = jnp.transpose(A_Wk, (1, 2, 0)).reshape(H * E, D)
    wvt = jnp.transpose(A_Wv, (1, 2, 0)).reshape(H * E, D)
    wo = A_Wo.reshape(H * E, D)
    any_spec = pl.BlockSpec(memory_space=pl.ANY)
    scratch = [
        pltpu.VMEM((S, D), BF),
        pltpu.VMEM((M, D), BF),
        pltpu.VMEM((H * E, D), BF),
        pltpu.VMEM((H * E, D), BF),
        pltpu.VMEM((H * E, D), BF),
        pltpu.VMEM((H * E, D), BF),
        pltpu.VMEM((D, D), BF),
        pltpu.VMEM((D, D), BF),
        pltpu.VMEM((D, F), BF),
        pltpu.VMEM((F, D), BF),
        pltpu.VMEM((NP, D // 2, PW), I32),
        pltpu.VMEM((NP, D // 2, PW), I32),
        pltpu.VMEM((NP, D // 2, PW), I32),
        pltpu.VMEM((NP, PW // 2, D), I32),
        pltpu.VMEM((D // 2, D), I32),
        pltpu.VMEM((D // 2, D), I32),
        pltpu.VMEM((D // 2, F), I32),
        pltpu.VMEM((F // 2, D), I32),
        pltpu.VMEM((S, D), F32),
        pltpu.VMEM((S, D), F32),
        pltpu.VMEM((D // 128, S + 2 * PAD, 128), F32),
        pltpu.VMEM((S, D), BF),
        pltpu.SemaphoreType.DMA((2,)),
        pltpu.SemaphoreType.DMA((4, NP)),
        pltpu.SemaphoreType.DMA((4,)),
        pltpu.SemaphoreType.DMA((S // RB,)),
    ]
    out = pl.pallas_call(
        _kernel,
        out_shape=jax.ShapeDtypeStruct((S, D), BF),
        in_specs=[any_spec] * 10,
        out_specs=any_spec,
        scratch_shapes=scratch,
        compiler_params=pltpu.CompilerParams(vmem_limit_bytes=120 * 1024 * 1024),
    )(x, mem0, wqt, wkt, wvt, wo, B_w1, B_w2, B_w3, B_w4)
    return out.reshape(1, S, D)


def pallas_interleave_layers__memory_aug_recurrent_mem_tr__mixer_s_mlp__prompt_kernel(
    A_x, A_mem0, A_Wq, A_Wk, A_Wv, A_Wo, A_seg_len, B_x, B_w1, B_w2, B_w3, B_w4,
):
    del B_x
    assert int(A_seg_len) == SEG and A_x.shape == (1, S, D)
    return _impl(A_x, A_mem0, A_Wq, A_Wk, A_Wv, A_Wo, B_w1, B_w2, B_w3, B_w4)
```

```python
import contextlib

import jax
import jax.numpy as jnp
from jax import lax
import jax.experimental.pallas as pl
import jax.experimental.pallas.tpu as pltpu

BF = jnp.bfloat16
F32 = jnp.float32
I32 = jnp.int32

S, D, H, E, M, SEG, F = 2048, 640, 32, 192, 8, 32, 1536
L = M + SEG
NSEG = S // SEG
NP = H // 2
PW = 2 * E
SCALE = float(E ** -0.5)
EPS = 1e-5
RB = 128
PAD = 8
GROUP = D // 4
XB = S // NP
WIN = 3
PROFILE = False
LAGS = (1, 4, 5)


def SCOPE(name):
    return jax.named_scope(name) if PROFILE else contextlib.nullcontext()


def _ln(x):
    m = jnp.mean(x, axis=-1, keepdims=True)
    c = x - m
    v = jnp.mean(c * c, axis=-1, keepdims=True)
    return c * lax.rsqrt(v + EPS)


def _gelu(x):
    k = 0.7978845608028654
    return 0.5 * x * (1.0 + jnp.tanh(k * (x + 0.044715 * (x * x * x))))


def _dot(a, b):
    return jnp.dot(a, b, preferred_element_type=F32)


def _unpack(w):
    return pltpu.bitcast(w, BF)


def _a_step(h, wq, wk, wv, wo):
    lane = lax.broadcasted_iota(I32, (L, 128), 1)
    lo = lane < 64
    col = lax.broadcasted_iota(I32, (L, 2 * L), 1)
    row = lax.broadcasted_iota(I32, (L, 2 * L), 0)
    first = col < L
    key = jnp.where(first, col, col - L)
    allowed = (row < M) | (row >= key)
    zt = jnp.zeros((L, 128), F32)
    q_, k_, v_, p_, o_ = {}, {}, {}, {}, {}
    acc = [None]

    def blockdiag(t):
        t0, t1, t2 = t[:, 0:128], t[:, 128:256], t[:, 256:384]
        top = jnp.concatenate([t0, jnp.where(lo, t1, 0.0), zt], axis=1)
        bot = jnp.concatenate([zt, jnp.where(lo, 0.0, t1), t2], axis=1)
        return jnp.concatenate([top, bot], axis=0).astype(BF)

    def qkv(p):
        q_[p] = _dot(h, _unpack(wq[p]))
        k_[p] = blockdiag(_dot(h, _unpack(wk[p])))
        v_[p] = blockdiag(_dot(h, _unpack(wv[p])))

    def qk(p):
        s = lax.dot_general(q_.pop(p), k_.pop(p), (((1,), (1,)), ((), ())),
                            preferred_element_type=F32)
        s = jnp.where(allowed, s * SCALE, -1e9)
        m1 = jnp.max(jnp.where(first, s, -jnp.inf), axis=1, keepdims=True)
        m2 = jnp.max(jnp.where(first, -jnp.inf, s), axis=1, keepdims=True)
        e = jnp.exp(s - jnp.where(first, m1, m2))
        l1 = jnp.sum(jnp.where(first, e, 0.0), axis=1, keepdims=True)
        l2 = jnp.sum(jnp.where(first, 0.0, e), axis=1, keepdims=True)
        p_[p] = e * pl.reciprocal(jnp.where(first, l1, l2), approx=False)

    def pv(p):
        o_[p] = _dot(p_.pop(p), v_.pop(p))

    def out(p):
        y = _dot(o_.pop(p), _unpack(wo[p]))
        acc[0] = y if acc[0] is None else acc[0] + y

    la, lb, lc = LAGS
    for t in range(NP + lc):
        if t < NP:
            qkv(t)
        if 0 <= t - la < NP:
            qk(t - la)
        if 0 <= t - lb < NP:
            pv(t - lb)
        if 0 <= t - lc < NP:
            out(t - lc)
    return acc[0]


def _shift_gather(hbuf, r0, rows):
    lane = lax.broadcasted_iota(I32, (rows, 128), 1)
    shifts = (-1, 1, -2, 2)
    tiles = []
    for t in range(D // 128):
        g_lo = (t * 128) // GROUP
        g_hi = (t * 128 + 127) // GROUP
        a = hbuf[t, pl.ds(r0 + PAD + shifts[g_lo], rows), :]
        if g_hi != g_lo:
            b = hbuf[t, pl.ds(r0 + PAD + shifts[g_hi], rows), :]
            a = jnp.where(lane < (g_hi * GROUP - t * 128), a, b)
        tiles.append(a)
    return jnp.concatenate(tiles, axis=1)


def _kernel(x_hbm, mem_hbm, wq_hbm, wk_hbm, wv_hbm, wo_hbm, w1_hbm, w2_hbm, w3_hbm, w4_hbm,
            o_hbm,
            xb, memb, sq, sk, sv, so, s1, s2, s3, s4,
            wq, wk, wv, wo, w1, w2, w3, w4,
            xres, xn, hbuf, ob, sem_x, sem_w, sem_b, sem_o):
    def mem_copy():
        return pltpu.make_async_copy(mem_hbm, memb, sem_x.at[0])

    def unit_copies(p):
        sl = pl.ds(pl.multiple_of(p * PW, PW), PW)
        xs = pl.ds(pl.multiple_of(p * XB, XB), XB)
        return [pltpu.make_async_copy(src.at[sl, :], dst.at[sl, :], sem_w.at[i, p])
                for i, (src, dst) in enumerate(((wq_hbm, sq), (wk_hbm, sk), (wv_hbm, sv),
                                                (wo_hbm, so)))] + [
            pltpu.make_async_copy(x_hbm.at[xs, :], xb.at[xs, :], sem_w.at[4, p])]

    def b_copy(i):
        src, dst = ((w1_hbm, s1), (w2_hbm, s2), (w3_hbm, s3), (w4_hbm, s4))[i]
        return pltpu.make_async_copy(src, dst, sem_b.at[i])

    mem_copy().start()
    for p in range(WIN):
        for cp in unit_copies(p):
            cp.start()

    hbuf[:, pl.ds(0, PAD), :] = jnp.zeros((D // 128, PAD, 128), F32)
    hbuf[:, pl.ds(PAD + S, PAD), :] = jnp.zeros((D // 128, PAD, 128), F32)

    def prep_unit(p, c):
        @pl.when(p + WIN < NP)
        def _():
            for cp in unit_copies(p + WIN):
                cp.start()

        cps = unit_copies(p)
        r0 = pl.multiple_of(p * PW, PW)
        for i, (src, dst) in enumerate(((sq, wq), (sk, wk), (sv, wv))):
            cps[i].wait()
            dst[p] = pltpu.bitcast(src[pl.ds(r0, PW), :].T, I32)
        cps[3].wait()
        wo[p] = pltpu.bitcast(so[pl.ds(r0, PW), :], I32)
        cps[4].wait()
        x0 = pl.multiple_of(p * XB, XB)
        x = xb[pl.ds(x0, XB), :].astype(F32)
        xres[pl.ds(x0, XB), :] = x
        xn[pl.ds(x0, XB), :] = _ln(x)
        return c
    with SCOPE('prep'):
        lax.fori_loop(0, NP, prep_unit, 0)
    for i in range(4):
        b_copy(i).start()
    mem_copy().wait()

    def out_copy(i):
        sl = pl.ds(pl.multiple_of(i * RB, RB), RB)
        return pltpu.make_async_copy(ob.at[sl, :], o_hbm.at[sl, :], sem_o.at[i])

    def layer(l, c):
        def seg_step(s, mem):
            r0 = pl.multiple_of(s * SEG, SEG)
            h = jnp.concatenate([mem, xn[pl.ds(r0, SEG), :]], axis=0)
            o = _a_step(h, wq, wk, wv, wo)
            xres[pl.ds(r0, SEG), :] = xres[pl.ds(r0, SEG), :] + o[M:, :]
            return o[:M, :]
        with SCOPE('A'):
            lax.fori_loop(0, NSEG, seg_step, memb[...].astype(F32))

        @pl.when(l == 0)
        def _():
            for i, (src, dst) in enumerate(((s1, w1), (s2, w2), (s3, w3), (s4, w4))):
                b_copy(i).wait()
                dst[...] = pltpu.bitcast(src[...], I32)

        def b1(i, c2):
            r0 = pl.multiple_of(i * RB, RB)
            xin = _ln(xres[pl.ds(r0, RB), :])
            xn[pl.ds(r0, RB), :] = xin
            hh = _gelu(_dot(_ln(xin), _unpack(w1[...])))
            for t in range(D // 128):
                hbuf[t, pl.ds(r0 + PAD, RB), :] = hh[:, t * 128:(t + 1) * 128]
            return c2
        with SCOPE('B1'):
            lax.fori_loop(0, S // RB, b1, 0)

        def b2(i, c2):
            r0 = pl.multiple_of(i * RB, RB)
            g = _shift_gather(hbuf, r0, RB)
            x1 = xn[pl.ds(r0, RB), :] + _dot(g, _unpack(w2[...]))
            u = _gelu(_dot(_ln(x1), _unpack(w3[...])))
            xo = xres[pl.ds(r0, RB), :] + (x1 + _dot(u, _unpack(w4[...])))
            xres[pl.ds(r0, RB), :] = xo
            xn[pl.ds(r0, RB), :] = _ln(xo)
            ob[pl.ds(r0, RB), :] = xo.astype(BF)

            @pl.when(l == 1)
            def _():
                out_copy(i).start()
            return c2
        with SCOPE('B2'):
            lax.fori_loop(0, S // RB, b2, 0)
        return c
    lax.fori_loop(0, 2, layer, 0)

    for i in range(S // RB):
        out_copy(i).wait()


@jax.jit
def _impl(A_x, A_mem0, A_Wq, A_Wk, A_Wv, A_Wo, B_w1, B_w2, B_w3, B_w4):
    x = A_x.reshape(S, D)
    mem0 = A_mem0.reshape(M, D)
    wqt = jnp.transpose(A_Wq, (1, 2, 0)).reshape(H * E, D)
    wkt = jnp.transpose(A_Wk, (1, 2, 0)).reshape(H * E, D)
    wvt = jnp.transpose(A_Wv, (1, 2, 0)).reshape(H * E, D)
    wo = A_Wo.reshape(H * E, D)
    any_spec = pl.BlockSpec(memory_space=pl.ANY)
    scratch = [
        pltpu.VMEM((S, D), BF),
        pltpu.VMEM((M, D), BF),
        pltpu.VMEM((H * E, D), BF),
        pltpu.VMEM((H * E, D), BF),
        pltpu.VMEM((H * E, D), BF),
        pltpu.VMEM((H * E, D), BF),
        pltpu.VMEM((D, D), BF),
        pltpu.VMEM((D, D), BF),
        pltpu.VMEM((D, F), BF),
        pltpu.VMEM((F, D), BF),
        pltpu.VMEM((NP, D // 2, PW), I32),
        pltpu.VMEM((NP, D // 2, PW), I32),
        pltpu.VMEM((NP, D // 2, PW), I32),
        pltpu.VMEM((NP, PW // 2, D), I32),
        pltpu.VMEM((D // 2, D), I32),
        pltpu.VMEM((D // 2, D), I32),
        pltpu.VMEM((D // 2, F), I32),
        pltpu.VMEM((F // 2, D), I32),
        pltpu.VMEM((S, D), F32),
        pltpu.VMEM((S, D), F32),
        pltpu.VMEM((D // 128, S + 2 * PAD, 128), F32),
        pltpu.VMEM((S, D), BF),
        pltpu.SemaphoreType.DMA((1,)),
        pltpu.SemaphoreType.DMA((5, NP)),
        pltpu.SemaphoreType.DMA((4,)),
        pltpu.SemaphoreType.DMA((S // RB,)),
    ]
    out = pl.pallas_call(
        _kernel,
        out_shape=jax.ShapeDtypeStruct((S, D), BF),
        in_specs=[any_spec] * 10,
        out_specs=any_spec,
        scratch_shapes=scratch,
        compiler_params=pltpu.CompilerParams(vmem_limit_bytes=120 * 1024 * 1024),
    )(x, mem0, wqt, wkt, wvt, wo, B_w1, B_w2, B_w3, B_w4)
    return out.reshape(1, S, D)


def pallas_interleave_layers__memory_aug_recurrent_mem_tr__mixer_s_mlp__prompt_kernel(
    A_x, A_mem0, A_Wq, A_Wk, A_Wv, A_Wo, A_seg_len, B_x, B_w1, B_w2, B_w3, B_w4,
):
    del B_x
    if isinstance(A_seg_len, int):
        assert A_seg_len == SEG
    assert A_x.shape == (1, S, D)
    return _impl(A_x, A_mem0, A_Wq, A_Wk, A_Wv, A_Wo, B_w1, B_w2, B_w3, B_w4)
```

```python
import contextlib

import jax
import jax.numpy as jnp
from jax import lax
import jax.experimental.pallas as pl
import jax.experimental.pallas.tpu as pltpu

BF = jnp.bfloat16
F32 = jnp.float32
I32 = jnp.int32

S, D, H, E, M, SEG, F = 2048, 640, 32, 192, 8, 32, 1536
L = M + SEG
NSEG = S // SEG
NP = H // 2
PW = 2 * E
SCALE = float(E ** -0.5)
EPS = 1e-5
U = 1
BR = SEG * U
NB = S // BR
HOOKS = {1: ((0, 1), (0, 3), (0, 7), (0, 10), (0, 13)),
         2: ((0, 1), (0, 4), (0, 10), (1, 2), (1, 9))}
PAD = 8
GROUP = D // 4
XB = S // NP
WIN = 3
PROFILE = False
LAGS = (1, 4, 5)


def SCOPE(name):
    return jax.named_scope(name) if PROFILE else contextlib.nullcontext()


def _ln(x):
    m = jnp.mean(x, axis=-1, keepdims=True)
    c = x - m
    v = jnp.mean(c * c, axis=-1, keepdims=True)
    return c * lax.rsqrt(v + EPS)


def _gelu(x):
    k = 0.7978845608028654
    return 0.5 * x * (1.0 + jnp.tanh(k * (x + 0.044715 * (x * x * x))))


def _dot(a, b):
    return jnp.dot(a, b, preferred_element_type=F32)


def _unpack(w):
    return pltpu.bitcast(w, BF)


def _a_step(h, wq, wk, wv, wo, hooks):
    lane = lax.broadcasted_iota(I32, (L, 128), 1)
    lo = lane < 64
    col = lax.broadcasted_iota(I32, (L, 2 * L), 1)
    row = lax.broadcasted_iota(I32, (L, 2 * L), 0)
    first = col < L
    key = jnp.where(first, col, col - L)
    allowed = (row < M) | (row >= key)
    zt = jnp.zeros((L, 128), F32)
    q_, k_, v_, p_, o_ = {}, {}, {}, {}, {}
    acc = [None]

    def blockdiag(t):
        t0, t1, t2 = t[:, 0:128], t[:, 128:256], t[:, 256:384]
        top = jnp.concatenate([t0, jnp.where(lo, t1, 0.0), zt], axis=1)
        bot = jnp.concatenate([zt, jnp.where(lo, 0.0, t1), t2], axis=1)
        return jnp.concatenate([top, bot], axis=0).astype(BF)

    def qkv(p):
        q_[p] = _dot(h, _unpack(wq[p]))
        k_[p] = blockdiag(_dot(h, _unpack(wk[p])))
        v_[p] = blockdiag(_dot(h, _unpack(wv[p])))

    def qk(p):
        s = lax.dot_general(q_.pop(p), k_.pop(p), (((1,), (1,)), ((), ())),
                            preferred_element_type=F32)
        s = jnp.where(allowed, s * SCALE, -1e9)
        m1 = jnp.max(jnp.where(first, s, -jnp.inf), axis=1, keepdims=True)
        m2 = jnp.max(jnp.where(first, -jnp.inf, s), axis=1, keepdims=True)
        e = jnp.exp(s - jnp.where(first, m1, m2))
        l1 = jnp.sum(jnp.where(first, e, 0.0), axis=1, keepdims=True)
        l2 = jnp.sum(jnp.where(first, 0.0, e), axis=1, keepdims=True)
        p_[p] = e * pl.reciprocal(jnp.where(first, l1, l2), approx=False)

    def pv(p):
        o_[p] = _dot(p_.pop(p), v_.pop(p))

    def out(p):
        y = _dot(o_.pop(p), _unpack(wo[p]))
        acc[0] = y if acc[0] is None else acc[0] + y

    la, lb, lc = LAGS
    for t in range(NP + lc):
        for fn in hooks.get(t, ()):
            fn()
        if t < NP:
            qkv(t)
        if 0 <= t - la < NP:
            qk(t - la)
        if 0 <= t - lb < NP:
            pv(t - lb)
        if 0 <= t - lc < NP:
            out(t - lc)
    return acc[0]


def _shift_gather(hbuf, r0, rows):
    lane = lax.broadcasted_iota(I32, (rows, 128), 1)
    shifts = (-1, 1, -2, 2)
    tiles = []
    for t in range(D // 128):
        g_lo = (t * 128) // GROUP
        g_hi = (t * 128 + 127) // GROUP
        a = hbuf[t, pl.ds(r0 + shifts[g_lo], rows), :]
        if g_hi != g_lo:
            b = hbuf[t, pl.ds(r0 + shifts[g_hi], rows), :]
            a = jnp.where(lane < (g_hi * GROUP - t * 128), a, b)
        tiles.append(a)
    return jnp.concatenate(tiles, axis=1)


def _kernel(x_hbm, mem_hbm, wq_hbm, wk_hbm, wv_hbm, wo_hbm, w1_hbm, w2_hbm, w3_hbm, w4_hbm,
            o_hbm,
            xb, memb, sq, sk, sv, so, s1, s2, s3, s4,
            wq, wk, wv, wo, w1, w2, w3, w4,
            xres, xn, hbuf, ob, sem_x, sem_w, sem_b, sem_o):
    def mem_copy():
        return pltpu.make_async_copy(mem_hbm, memb, sem_x.at[0])

    def unit_copies(p):
        sl = pl.ds(pl.multiple_of(p * PW, PW), PW)
        xs = pl.ds(pl.multiple_of(p * XB, XB), XB)
        return [pltpu.make_async_copy(src.at[sl, :], dst.at[sl, :], sem_w.at[i, p])
                for i, (src, dst) in enumerate(((wq_hbm, sq), (wk_hbm, sk), (wv_hbm, sv),
                                                (wo_hbm, so)))] + [
            pltpu.make_async_copy(x_hbm.at[xs, :], xb.at[xs, :], sem_w.at[4, p])]

    def b_copy(i):
        src, dst = ((w1_hbm, s1), (w2_hbm, s2), (w3_hbm, s3), (w4_hbm, s4))[i]
        return pltpu.make_async_copy(src, dst, sem_b.at[i])

    mem_copy().start()
    for p in range(WIN):
        for cp in unit_copies(p):
            cp.start()

    hbuf[:, pl.ds(0, PAD), :] = jnp.zeros((D // 128, PAD, 128), F32)
    hbuf[:, pl.ds(PAD + S, 3 * PAD + BR), :] = jnp.zeros((D // 128, 3 * PAD + BR, 128), F32)
    xres[pl.ds(S, BR), :] = jnp.zeros((BR, D), F32)
    xn[pl.ds(S, BR), :] = jnp.zeros((BR, D), F32)
    for w in (w1, w2, w3, w4):
        w[...] = jnp.zeros(w.shape, I32)

    def prep_unit(p, c):
        @pl.when(p + WIN < NP)
        def _():
            for cp in unit_copies(p + WIN):
                cp.start()

        cps = unit_copies(p)
        r0 = pl.multiple_of(p * PW, PW)
        for i, (src, dst) in enumerate(((sq, wq), (sk, wk), (sv, wv))):
            cps[i].wait()
            dst[p] = pltpu.bitcast(src[pl.ds(r0, PW), :].T, I32)
        cps[3].wait()
        wo[p] = pltpu.bitcast(so[pl.ds(r0, PW), :], I32)
        cps[4].wait()
        x0 = pl.multiple_of(p * XB, XB)
        x = xb[pl.ds(x0, XB), :].astype(F32)
        xres[pl.ds(x0, XB), :] = x
        xn[pl.ds(x0, XB), :] = _ln(x)
        return c
    with SCOPE('prep'):
        lax.fori_loop(0, NP, prep_unit, 0)
    for i in range(4):
        b_copy(i).start()
    mem_copy().wait()

    def b_rows(jb):
        valid = jb >= 0
        blk = lax.rem(jnp.maximum(jb, 0), NB)
        r0 = pl.multiple_of(jnp.where(valid, blk * BR, S), BR)
        h0 = pl.multiple_of(jnp.where(valid, blk * BR + PAD, S + 3 * PAD), PAD)
        return r0, h0

    def b1_stages(jb):
        r0, h0 = b_rows(jb)
        st = {}

        def s_ln():
            xin = _ln(xres[pl.ds(r0, BR), :])
            xn[pl.ds(r0, BR), :] = xin
            st['t'] = _ln(xin)

        def s_w1():
            hh = _gelu(_dot(st.pop('t'), _unpack(w1[...])))
            for t in range(D // 128):
                hbuf[t, pl.ds(h0, BR), :] = hh[:, t * 128:(t + 1) * 128]
        return [s_ln, s_w1]

    def b2_stages(jb):
        r0, h0 = b_rows(jb)
        st = {}

        def s_w2():
            g = _shift_gather(hbuf, h0, BR)
            x1 = xn[pl.ds(r0, BR), :] + _dot(g, _unpack(w2[...]))
            st['x1'] = x1
            st['u'] = _ln(x1)

        def s_w3():
            st['g'] = _gelu(_dot(st.pop('u'), _unpack(w3[...])))

        def s_w4():
            xo = xres[pl.ds(r0, BR), :] + (st.pop('x1') + _dot(st.pop('g'), _unpack(w4[...])))
            xres[pl.ds(r0, BR), :] = xo
            xn[pl.ds(r0, BR), :] = _ln(xo)
            ob[pl.ds(r0, BR), :] = xo.astype(BF)
        return [s_w2, s_w3, s_w4]

    def out_copy(blk):
        sl = pl.ds(pl.multiple_of(blk * BR, BR), BR)
        return pltpu.make_async_copy(ob.at[sl, :], o_hbm.at[sl, :], sem_o.at[0])

    mem0 = memb[...].astype(F32)

    def step(j, mem):
        @pl.when(j == 1)
        def _():
            b_copy(0).wait()
            w1[...] = pltpu.bitcast(s1[...], I32)

        @pl.when(j == 2)
        def _():
            for i, (src, dst) in ((1, (s2, w2)), (2, (s3, w3)), (3, (s4, w4))):
                b_copy(i).wait()
                dst[...] = pltpu.bitcast(src[...], I32)

        stages = b1_stages(j - 1) + b2_stages(j - 2)
        for u in range(U):
            s = lax.rem(j, NB) * U + u
            r0 = pl.multiple_of(s * SEG, SEG)
            if u == 0:
                mem = jnp.where(s == 0, memb[...].astype(F32), mem)
            hooks = {}
            for k, (uu, t) in enumerate(HOOKS[U]):
                if uu == u:
                    hooks.setdefault(t, []).append(stages[k])
            h = jnp.concatenate([mem, xn[pl.ds(r0, SEG), :]], axis=0)
            o = _a_step(h, wq, wk, wv, wo, hooks)
            xres[pl.ds(r0, SEG), :] = xres[pl.ds(r0, SEG), :] + o[M:, :]
            mem = o[:M, :]

        @pl.when(j - 2 >= NB)
        def _():
            out_copy(j - 2 - NB).start()
        return mem

    with SCOPE('main'):
        lax.fori_loop(0, 2 * NB, step, mem0)

    with SCOPE('epilogue'):
        last = 2 * NB - 1
        for fn in b1_stages(last) + b2_stages(last - 1):
            fn()
        out_copy(NB - 2).start()
        for fn in b2_stages(last):
            fn()
        out_copy(NB - 1).start()
    pltpu.make_async_copy(ob.at[pl.ds(0, S), :], o_hbm, sem_o.at[0]).wait()


@jax.jit
def _impl(A_x, A_mem0, A_Wq, A_Wk, A_Wv, A_Wo, B_w1, B_w2, B_w3, B_w4):
    x = A_x.reshape(S, D)
    mem0 = A_mem0.reshape(M, D)
    wqt = jnp.transpose(A_Wq, (1, 2, 0)).reshape(H * E, D)
    wkt = jnp.transpose(A_Wk, (1, 2, 0)).reshape(H * E, D)
    wvt = jnp.transpose(A_Wv, (1, 2, 0)).reshape(H * E, D)
    wo = A_Wo.reshape(H * E, D)
    any_spec = pl.BlockSpec(memory_space=pl.ANY)
    scratch = [
        pltpu.VMEM((S, D), BF),
        pltpu.VMEM((M, D), BF),
        pltpu.VMEM((H * E, D), BF),
        pltpu.VMEM((H * E, D), BF),
        pltpu.VMEM((H * E, D), BF),
        pltpu.VMEM((H * E, D), BF),
        pltpu.VMEM((D, D), BF),
        pltpu.VMEM((D, D), BF),
        pltpu.VMEM((D, F), BF),
        pltpu.VMEM((F, D), BF),
        pltpu.VMEM((NP, D // 2, PW), I32),
        pltpu.VMEM((NP, D // 2, PW), I32),
        pltpu.VMEM((NP, D // 2, PW), I32),
        pltpu.VMEM((NP, PW // 2, D), I32),
        pltpu.VMEM((D // 2, D), I32),
        pltpu.VMEM((D // 2, D), I32),
        pltpu.VMEM((D // 2, F), I32),
        pltpu.VMEM((F // 2, D), I32),
        pltpu.VMEM((S + BR, D), F32),
        pltpu.VMEM((S + BR, D), F32),
        pltpu.VMEM((D // 128, S + 4 * PAD + BR, 128), F32),
        pltpu.VMEM((S + BR, D), BF),
        pltpu.SemaphoreType.DMA((1,)),
        pltpu.SemaphoreType.DMA((5, NP)),
        pltpu.SemaphoreType.DMA((4,)),
        pltpu.SemaphoreType.DMA((1,)),
    ]
    out = pl.pallas_call(
        _kernel,
        out_shape=jax.ShapeDtypeStruct((S, D), BF),
        in_specs=[any_spec] * 10,
        out_specs=any_spec,
        scratch_shapes=scratch,
        compiler_params=pltpu.CompilerParams(vmem_limit_bytes=120 * 1024 * 1024),
    )(x, mem0, wqt, wkt, wvt, wo, B_w1, B_w2, B_w3, B_w4)
    return out.reshape(1, S, D)


def pallas_interleave_layers__memory_aug_recurrent_mem_tr__mixer_s_mlp__prompt_kernel(
    A_x, A_mem0, A_Wq, A_Wk, A_Wv, A_Wo, A_seg_len, B_x, B_w1, B_w2, B_w3, B_w4,
):
    del B_x
    if isinstance(A_seg_len, int):
        assert A_seg_len == SEG
    assert A_x.shape == (1, S, D)
    return _impl(A_x, A_mem0, A_Wq, A_Wk, A_Wv, A_Wo, B_w1, B_w2, B_w3, B_w4)
```

```python
import contextlib

import jax
import jax.numpy as jnp
from jax import lax
import jax.experimental.pallas as pl
import jax.experimental.pallas.tpu as pltpu

BF = jnp.bfloat16
F32 = jnp.float32
I32 = jnp.int32

S, D, H, E, M, SEG, F = 2048, 640, 32, 192, 8, 32, 1536
L = M + SEG
NSEG = S // SEG
NP = H // 2
PW = 2 * E
SCALE = float(E ** -0.5)
EPS = 1e-5
TK = 24
LA = S - NSEG * TK
RING = LA + SEG
BR = SEG
NB = S // BR
PAD = 8
GROUP = D // 4
XB = 128
NSL = 3
LAGS = (1, 4, 5)
HOOKS = (1, 3, 7, 10, 13)
PRE_UNROLL = 2
B_PACKED = True
PROFILE = False


def SCOPE(name):
    return jax.named_scope(name) if PROFILE else contextlib.nullcontext()


def _ln(x):
    m = jnp.mean(x, axis=-1, keepdims=True)
    c = x - m
    v = jnp.mean(c * c, axis=-1, keepdims=True)
    return c * lax.rsqrt(v + EPS)


def _gelu(x):
    k = 0.7978845608028654
    return 0.5 * x * (1.0 + jnp.tanh(k * (x + 0.044715 * (x * x * x))))


def _dot(a, b):
    return jnp.dot(a, b, preferred_element_type=F32)


def _unpack(w):
    return w if w.dtype == BF else pltpu.bitcast(w, BF)


def _a_step(h, rd, wr, wq, wk, wv, wo, rq, rk, rv, hooks):
    lane = lax.broadcasted_iota(I32, (L, 128), 1)
    lo = lane < 64
    col = lax.broadcasted_iota(I32, (L, 2 * L), 1)
    row = lax.broadcasted_iota(I32, (L, 2 * L), 0)
    first = col < L
    key = jnp.where(first, col, col - L)
    allowed = (row < M) | (row >= key)
    zt = jnp.zeros((L, 128), F32)
    q_, k_, v_, p_, o_ = {}, {}, {}, {}, {}
    acc = [None]

    def blockdiag(t):
        t0, t1, t2 = t[:, 0:128], t[:, 128:256], t[:, 256:384]
        top = jnp.concatenate([t0, jnp.where(lo, t1, 0.0), zt], axis=1)
        bot = jnp.concatenate([zt, jnp.where(lo, 0.0, t1), t2], axis=1)
        return jnp.concatenate([top, bot], axis=0).astype(BF)

    def project(w, ring, p):
        y = _dot(h, _unpack(w[p]))
        for i, r in enumerate(wr):
            ring[p, pl.ds(r, 8), :] = y[M + 8 * i:M + 8 * i + 8, :]
        return y[:M, :]

    def qkv(p):
        q_[p] = project(wq, rq, p)
        k_[p] = project(wk, rk, p)
        v_[p] = project(wv, rv, p)

    def full(mem_rows, ring, p):
        return jnp.concatenate([mem_rows, ring[p, pl.ds(rd, SEG), :]], axis=0)

    def load_qk(p):
        q_[p] = full(q_[p], rq, p)
        k_[p] = blockdiag(full(k_[p], rk, p))

    def load_v(p):
        v_[p] = blockdiag(full(v_[p], rv, p))

    def qk(p):
        s = lax.dot_general(q_.pop(p), k_.pop(p), (((1,), (1,)), ((), ())),
                            preferred_element_type=F32)
        s = jnp.where(allowed, s * SCALE, -1e9)
        m1 = jnp.max(jnp.where(first, s, -jnp.inf), axis=1, keepdims=True)
        m2 = jnp.max(jnp.where(first, -jnp.inf, s), axis=1, keepdims=True)
        e = jnp.exp(s - jnp.where(first, m1, m2))
        l1 = jnp.sum(jnp.where(first, e, 0.0), axis=1, keepdims=True)
        l2 = jnp.sum(jnp.where(first, 0.0, e), axis=1, keepdims=True)
        p_[p] = e * pl.reciprocal(jnp.where(first, l1, l2), approx=False)

    def pv(p):
        o_[p] = _dot(p_.pop(p), v_.pop(p))

    def out(p):
        y = _dot(o_.pop(p), _unpack(wo[p]))
        acc[0] = y if acc[0] is None else acc[0] + y

    la, lb, lc = LAGS
    for t in range(NP + lc):
        for fn in hooks.get(t, ()):
            fn()
        if 0 <= t - la < NP:
            load_qk(t - la)
        if 0 <= t - lb < NP:
            load_v(t - lb)
        if t < NP:
            qkv(t)
        if 0 <= t - la < NP:
            qk(t - la)
        if 0 <= t - lb < NP:
            pv(t - lb)
        if 0 <= t - lc < NP:
            out(t - lc)
    return acc[0]


def _shift_gather(hbuf, r0, rows):
    lane = lax.broadcasted_iota(I32, (rows, 128), 1)
    shifts = (-1, 1, -2, 2)
    tiles = []
    for t in range(D // 128):
        g_lo = (t * 128) // GROUP
        g_hi = (t * 128 + 127) // GROUP
        a = hbuf[t, pl.ds(r0 + shifts[g_lo], rows), :]
        if g_hi != g_lo:
            b = hbuf[t, pl.ds(r0 + shifts[g_hi], rows), :]
            a = jnp.where(lane < (g_hi * GROUP - t * 128), a, b)
        tiles.append(a)
    return jnp.concatenate(tiles, axis=1)


def _kernel(x_hbm, mem_hbm, wq_hbm, wk_hbm, wv_hbm, wo_hbm, w1_hbm, w2_hbm, w3_hbm, w4_hbm,
            o_hbm,
            xb, memb, sq, sk, sv, so, s1, s2, s3, s4,
            wq, wk, wv, wo, w1, w2, w3, w4,
            xres, xn, hbuf, ob, rq, rk, rv, xa, tmp0, tmp1, sem_x, sem_w, sem_b, sem_o):
    NXH = LA // XB

    def head_copies():
        return [pltpu.make_async_copy(mem_hbm, memb, sem_x.at[0]),
                pltpu.make_async_copy(x_hbm.at[pl.ds(0, LA), :], xb.at[pl.ds(0, LA), :],
                                      sem_x.at[1])]

    def unit_copies(p):
        sl = pl.ds(pl.multiple_of(p * PW, PW), PW)
        slot = lax.rem(p, NSL)
        return [pltpu.make_async_copy(src.at[sl, :], dst.at[slot], sem_w.at[i, p])
                for i, (src, dst) in enumerate(((wq_hbm, sq), (wk_hbm, sk), (wv_hbm, sv),
                                                (wo_hbm, so)))]

    def xblk_copy(b):
        xs = pl.ds(pl.multiple_of(b * XB, XB), XB)
        return pltpu.make_async_copy(x_hbm.at[xs, :], xb.at[xs, :], sem_w.at[4, b])

    def b_copies():
        return [pltpu.make_async_copy(src, dst, sem_b.at[i])
                for i, (src, dst) in enumerate(((w1_hbm, s1), (w2_hbm, s2), (w3_hbm, s3),
                                                (w4_hbm, s4)))]

    def init_rows(x0, ln_dst, ln0):
        x = xb[pl.ds(x0, XB), :].astype(F32)
        xres[pl.ds(x0, XB), :] = x
        ln_dst[pl.ds(ln0, XB), :] = _ln(x)

    def relayout(p, tmp):
        slot = lax.rem(p, NSL)
        for i, (src, dst) in enumerate(((sq, wq), (sk, wk), (sv, wv))):
            t = pltpu.bitcast(src[slot].T, I32)
            dst[p] = t
            tmp[i] = t
        wo[p] = pltpu.bitcast(so[slot], I32)

    def project_ahead(p, src, weights):
        for w, ring in zip(weights, (rq, rk, rv)):
            for c in range(LA // 128):
                t = src[c * 128:(c + 1) * 128, :]
                ring[p, c * 128:(c + 1) * 128, :] = _dot(t, _unpack(w()))

    for cp in head_copies() + unit_copies(0):
        cp.start()

    hbuf[:, pl.ds(0, PAD), :] = jnp.zeros((D // 128, PAD, 128), F32)
    hbuf[:, pl.ds(PAD + S, 3 * PAD + BR), :] = jnp.zeros((D // 128, 3 * PAD + BR, 128), F32)
    xres[pl.ds(S, BR), :] = jnp.zeros((BR, D), F32)
    xn[pl.ds(S, BR), :] = jnp.zeros((BR, D), F32)

    def start_unit(u):
        @pl.when(u < NP)
        def _():
            for cp in unit_copies(u):
                cp.start()

        @pl.when(u + NXH - 1 < S // XB)
        def _():
            xblk_copy(u + NXH - 1).start()

        @pl.when(u == NP)
        def _():
            for cp in b_copies():
                cp.start()

    with SCOPE('head'):
        for cp in head_copies() + unit_copies(0):
            cp.wait()
        start_unit(1)

        def head_rows(b, c):
            x0 = pl.multiple_of(b * XB, XB)
            init_rows(x0, xa, x0)
            return c
        lax.fori_loop(0, NXH, head_rows, 0)
        relayout(0, tmp0)
        start_unit(2)

    def prep_unit(p, cur, nxt):
        @pl.when(p + 1 < NP)
        def _():
            for cp in unit_copies(p + 1):
                cp.wait()

        @pl.when(p + NXH < S // XB)
        def _():
            xblk_copy(p + NXH).wait()

        relayout(jnp.minimum(p + 1, NP - 1), nxt)
        x0 = pl.multiple_of(jnp.minimum(p + NXH, S // XB - 1) * XB, XB)
        init_rows(x0, xn, x0)
        project_ahead(p, xa, [lambda i=i: cur[i] for i in range(3)])
        start_unit(p + 3)

    def prep_two(pp, c):
        prep_unit(2 * pp, tmp0, tmp1)
        prep_unit(2 * pp + 1, tmp1, tmp0)
        return c
    with SCOPE('prep'):
        lax.fori_loop(0, NP // 2, prep_two, 0)

    with SCOPE('bprep'):
        for cp in b_copies():
            cp.wait()
        if B_PACKED:
            for src, dst in ((s1, w1), (s2, w2), (s3, w3), (s4, w4)):
                dst[...] = pltpu.bitcast(src[...], I32)
        else:
            w1, w2, w3, w4 = s1, s2, s3, s4

    def b_rows(jb):
        valid = jb >= 0
        blk = lax.rem(jnp.maximum(jb, 0), NB)
        r0 = pl.multiple_of(jnp.where(valid, blk * BR, S), BR)
        h0 = pl.multiple_of(jnp.where(valid, blk * BR + PAD, S + 3 * PAD), PAD)
        return r0, h0

    def b1_stages(jb):
        r0, h0 = b_rows(jb)
        st = {}

        def s_ln():
            xin = _ln(xres[pl.ds(r0, BR), :])
            xn[pl.ds(r0, BR), :] = xin
            st['t'] = _ln(xin)

        def s_w1():
            hh = _gelu(_dot(st.pop('t'), _unpack(w1[...])))
            for t in range(D // 128):
                hbuf[t, pl.ds(h0, BR), :] = hh[:, t * 128:(t + 1) * 128]
        return [s_ln, s_w1]

    def b2_stages(jb):
        r0, h0 = b_rows(jb)
        st = {}

        def s_w2():
            g = _shift_gather(hbuf, h0, BR)
            x1 = xn[pl.ds(r0, BR), :] + _dot(g, _unpack(w2[...]))
            st['x1'] = x1
            st['u'] = _ln(x1)

        def s_w3():
            st['g'] = _gelu(_dot(st.pop('u'), _unpack(w3[...])))

        def s_w4():
            xo = xres[pl.ds(r0, BR), :] + (st.pop('x1') + _dot(st.pop('g'), _unpack(w4[...])))
            xres[pl.ds(r0, BR), :] = xo
            xn[pl.ds(r0, BR), :] = _ln(xo)
            ob[pl.ds(r0, BR), :] = xo.astype(BF)
        return [s_w2, s_w3, s_w4]

    def out_copy(blk):
        sl = pl.ds(pl.multiple_of(blk * BR, BR), BR)
        return pltpu.make_async_copy(ob.at[sl, :], o_hbm.at[sl, :], sem_o.at[0])

    def step(j, mem):
        @pl.when(j == NSEG)
        def _():
            lax.fori_loop(0, NP, lambda p, c: (project_ahead(
                p, xn, [lambda w=w: w[p] for w in (wq, wk, wv)]), c)[1], 0, unroll=PRE_UNROLL)

        stages = b1_stages(j - 1) + b2_stages(j - 2)
        hooks = {t: [fn] for t, fn in zip(HOOKS, stages)}
        s = lax.rem(j, NSEG)
        mem = jnp.where(s == 0, memb[...].astype(F32), mem)
        r0 = pl.multiple_of(s * SEG, SEG)
        n0 = pl.multiple_of(LA + s * TK, 8)
        rd = pl.multiple_of(lax.rem(r0, RING), SEG)
        wr = [pl.multiple_of(lax.rem(n0 + 8 * i, RING), 8) for i in range(TK // 8)]
        h = jnp.concatenate([mem, xn[pl.ds(n0, TK), :]], axis=0)
        o = _a_step(h, rd, wr, wq, wk, wv, wo, rq, rk, rv, hooks)
        xres[pl.ds(r0, SEG), :] = xres[pl.ds(r0, SEG), :] + o[M:, :]

        @pl.when(j - 2 >= NB)
        def _():
            out_copy(j - 2 - NB).start()
        return o[:M, :]

    with SCOPE('main'):
        lax.fori_loop(0, 2 * NSEG, step, memb[...].astype(F32))

    with SCOPE('epilogue'):
        last = 2 * NB - 1
        for fn in b1_stages(last) + b2_stages(last - 1):
            fn()
        out_copy(NB - 2).start()
        for fn in b2_stages(last):
            fn()
        out_copy(NB - 1).start()
    pltpu.make_async_copy(ob.at[pl.ds(0, S), :], o_hbm, sem_o.at[0]).wait()


@jax.jit
def _impl(A_x, A_mem0, A_Wq, A_Wk, A_Wv, A_Wo, B_w1, B_w2, B_w3, B_w4):
    x = A_x.reshape(S, D)
    mem0 = A_mem0.reshape(M, D)
    wqt = jnp.transpose(A_Wq, (1, 2, 0)).reshape(H * E, D)
    wkt = jnp.transpose(A_Wk, (1, 2, 0)).reshape(H * E, D)
    wvt = jnp.transpose(A_Wv, (1, 2, 0)).reshape(H * E, D)
    wo = A_Wo.reshape(H * E, D)
    any_spec = pl.BlockSpec(memory_space=pl.ANY)
    scratch = [
        pltpu.VMEM((S, D), BF),
        pltpu.VMEM((M, D), BF),
        pltpu.VMEM((NSL, PW, D), BF),
        pltpu.VMEM((NSL, PW, D), BF),
        pltpu.VMEM((NSL, PW, D), BF),
        pltpu.VMEM((NSL, PW, D), BF),
        pltpu.VMEM((D, D), BF),
        pltpu.VMEM((D, D), BF),
        pltpu.VMEM((D, F), BF),
        pltpu.VMEM((F, D), BF),
        pltpu.VMEM((NP, D // 2, PW), I32),
        pltpu.VMEM((NP, D // 2, PW), I32),
        pltpu.VMEM((NP, D // 2, PW), I32),
        pltpu.VMEM((NP, PW // 2, D), I32),
        pltpu.VMEM((D // 2, D), I32),
        pltpu.VMEM((D // 2, D), I32),
        pltpu.VMEM((D // 2, F), I32),
        pltpu.VMEM((F // 2, D), I32),
        pltpu.VMEM((S + BR, D), F32),
        pltpu.VMEM((S + BR, D), F32),
        pltpu.VMEM((D // 128, S + 4 * PAD + BR, 128), F32),
        pltpu.VMEM((S + BR, D), BF),
        pltpu.VMEM((NP, RING, PW), F32),
        pltpu.VMEM((NP, RING, PW), F32),
        pltpu.VMEM((NP, RING, PW), F32),
        pltpu.VMEM((LA, D), F32),
        pltpu.VMEM((3, D // 2, PW), I32),
        pltpu.VMEM((3, D // 2, PW), I32),
        pltpu.SemaphoreType.DMA((2,)),
        pltpu.SemaphoreType.DMA((5, NP)),
        pltpu.SemaphoreType.DMA((4,)),
        pltpu.SemaphoreType.DMA((1,)),
    ]
    out = pl.pallas_call(
        _kernel,
        out_shape=jax.ShapeDtypeStruct((S, D), BF),
        in_specs=[any_spec] * 10,
        out_specs=any_spec,
        scratch_shapes=scratch,
        compiler_params=pltpu.CompilerParams(vmem_limit_bytes=126 * 1024 * 1024),
    )(x, mem0, wqt, wkt, wvt, wo, B_w1, B_w2, B_w3, B_w4)
    return out.reshape(1, S, D)


def pallas_interleave_layers__memory_aug_recurrent_mem_tr__mixer_s_mlp__prompt_kernel(
    A_x, A_mem0, A_Wq, A_Wk, A_Wv, A_Wo, A_seg_len, B_x, B_w1, B_w2, B_w3, B_w4,
):
    del B_x
    if isinstance(A_seg_len, int):
        assert A_seg_len == SEG
    assert A_x.shape == (1, S, D)
    return _impl(A_x, A_mem0, A_Wq, A_Wk, A_Wv, A_Wo, B_w1, B_w2, B_w3, B_w4)
```

```python
import contextlib

import jax
import jax.numpy as jnp
from jax import lax
import jax.experimental.pallas as pl
import jax.experimental.pallas.tpu as pltpu

BF = jnp.bfloat16
F32 = jnp.float32
I32 = jnp.int32

S, D, H, E, M, SEG, F = 2048, 640, 32, 192, 8, 32, 1536
L = M + SEG
NSEG = S // SEG
NP = H // 2
PW = 2 * E
SCALE = float(E ** -0.5)
EPS = 1e-5
TK = 24
LA = S - NSEG * TK
RING = LA + SEG
BR = SEG
NB = S // BR
PAD = 8
GROUP = D // 4
XB = 128
NSL = 3
LAGS = (2, 4, 6)
HOOKS = ((1, 3, 7, 10, 13),) + ((1, 3, 7, 14, 99),) * 7
PRE_UNROLL = 2
UNROLL = 2
B_PACKED = True
PROFILE = False


def SCOPE(name):
    return jax.named_scope(name) if PROFILE else contextlib.nullcontext()


def _ln(x):
    m = jnp.mean(x, axis=-1, keepdims=True)
    c = x - m
    v = jnp.mean(c * c, axis=-1, keepdims=True)
    return c * lax.rsqrt(v + EPS)


def _gelu(x):
    k = 0.7978845608028654
    return 0.5 * x * (1.0 + jnp.tanh(k * (x + 0.044715 * (x * x * x))))


def _dot(a, b):
    return jnp.dot(a, b, preferred_element_type=F32)


def _unpack(w):
    return w if w.dtype == BF else pltpu.bitcast(w, BF)


def _a_step(h, rd, wr, wq, wk, wv, wo, rq, rk, rv, hooks):
    lane = lax.broadcasted_iota(I32, (L, 128), 1)
    lo = lane < 64
    col = lax.broadcasted_iota(I32, (L, 2 * L), 1)
    row = lax.broadcasted_iota(I32, (L, 2 * L), 0)
    first = col < L
    key = jnp.where(first, col, col - L)
    allowed = (row < M) | (row >= key)
    zt = jnp.zeros((L, 128), F32)
    q_, k_, v_, p_, o_ = {}, {}, {}, {}, {}
    acc = [None]

    def blockdiag(t):
        t0, t1, t2 = t[:, 0:128], t[:, 128:256], t[:, 256:384]
        top = jnp.concatenate([t0, jnp.where(lo, t1, 0.0), zt], axis=1)
        bot = jnp.concatenate([zt, jnp.where(lo, 0.0, t1), t2], axis=1)
        return jnp.concatenate([top, bot], axis=0).astype(BF)

    def project(w, ring, p):
        y = _dot(h, _unpack(w[p]))
        for i, r in enumerate(wr):
            ring[p, pl.ds(r, 8), :] = y[M + 8 * i:M + 8 * i + 8, :]
        return y[:M, :]

    def qkv(p):
        q_[p] = project(wq, rq, p)
        k_[p] = project(wk, rk, p)
        v_[p] = project(wv, rv, p)

    def full(mem_rows, ring, p):
        return jnp.concatenate([mem_rows, ring[p, pl.ds(rd, SEG), :]], axis=0)

    def load_qk(p):
        q_[p] = full(q_[p], rq, p)
        k_[p] = blockdiag(full(k_[p], rk, p))

    def load_v(p):
        v_[p] = blockdiag(full(v_[p], rv, p))

    def qk(p):
        s = lax.dot_general(q_.pop(p), k_.pop(p), (((1,), (1,)), ((), ())),
                            preferred_element_type=F32)
        s = jnp.where(allowed, s * SCALE, -1e9)
        m1 = jnp.max(jnp.where(first, s, -jnp.inf), axis=1, keepdims=True)
        m2 = jnp.max(jnp.where(first, -jnp.inf, s), axis=1, keepdims=True)
        e = jnp.exp(s - jnp.where(first, m1, m2))
        l1 = jnp.sum(jnp.where(first, e, 0.0), axis=1, keepdims=True)
        l2 = jnp.sum(jnp.where(first, 0.0, e), axis=1, keepdims=True)
        p_[p] = e * pl.reciprocal(jnp.where(first, l1, l2), approx=False)

    def pv(p):
        o_[p] = _dot(p_.pop(p), v_.pop(p))

    def out(p):
        y = _dot(o_.pop(p), _unpack(wo[p]))
        acc[0] = y if acc[0] is None else acc[0] + y

    la, lb, lc = LAGS
    for t in range(NP + lc):
        for fn in hooks.get(t, ()):
            fn()
        if 0 <= t - la < NP:
            load_qk(t - la)
        if 0 <= t - lb < NP:
            load_v(t - lb)
        if t < NP:
            qkv(t)
        if 0 <= t - la < NP:
            qk(t - la)
        if 0 <= t - lb < NP:
            pv(t - lb)
        if 0 <= t - lc < NP:
            out(t - lc)
    for fn in hooks.get(99, ()):
        fn()
    return acc[0]


def _shift_gather(hbuf, r0, rows):
    lane = lax.broadcasted_iota(I32, (rows, 128), 1)
    shifts = (-1, 1, -2, 2)
    tiles = []
    for t in range(D // 128):
        g_lo = (t * 128) // GROUP
        g_hi = (t * 128 + 127) // GROUP
        a = hbuf[t, pl.ds(r0 + shifts[g_lo], rows), :]
        if g_hi != g_lo:
            b = hbuf[t, pl.ds(r0 + shifts[g_hi], rows), :]
            a = jnp.where(lane < (g_hi * GROUP - t * 128), a, b)
        tiles.append(a)
    return jnp.concatenate(tiles, axis=1)


def _kernel(x_hbm, mem_hbm, wq_hbm, wk_hbm, wv_hbm, wo_hbm, w1_hbm, w2_hbm, w3_hbm, w4_hbm,
            o_hbm,
            xb, memb, sq, sk, sv, so, s1, s2, s3, s4,
            wq, wk, wv, wo, w1, w2, w3, w4,
            xres, xn, hbuf, ob, rq, rk, rv, xa, tmp0, tmp1, sem_x, sem_w, sem_b, sem_o):
    NXH = LA // XB

    def head_copies():
        return [pltpu.make_async_copy(mem_hbm, memb, sem_x.at[0]),
                pltpu.make_async_copy(x_hbm.at[pl.ds(0, LA), :], xb.at[pl.ds(0, LA), :],
                                      sem_x.at[1])]

    def unit_copies(p):
        sl = pl.ds(pl.multiple_of(p * PW, PW), PW)
        slot = lax.rem(p, NSL)
        return [pltpu.make_async_copy(src.at[sl, :], dst.at[slot], sem_w.at[i, p])
                for i, (src, dst) in enumerate(((wq_hbm, sq), (wk_hbm, sk), (wv_hbm, sv),
                                                (wo_hbm, so)))]

    def xblk_copy(b):
        xs = pl.ds(pl.multiple_of(b * XB, XB), XB)
        return pltpu.make_async_copy(x_hbm.at[xs, :], xb.at[xs, :], sem_w.at[4, b])

    def b_copies():
        return [pltpu.make_async_copy(src, dst, sem_b.at[i])
                for i, (src, dst) in enumerate(((w1_hbm, s1), (w2_hbm, s2), (w3_hbm, s3),
                                                (w4_hbm, s4)))]

    def init_rows(x0, ln_dst, ln0):
        x = xb[pl.ds(x0, XB), :].astype(F32)
        xres[pl.ds(x0, XB), :] = x
        ln_dst[pl.ds(ln0, XB), :] = _ln(x)

    def relayout(p, tmp):
        slot = lax.rem(p, NSL)
        for i, (src, dst) in enumerate(((sq, wq), (sk, wk), (sv, wv))):
            t = pltpu.bitcast(src[slot].T, I32)
            dst[p] = t
            tmp[i] = t
        wo[p] = pltpu.bitcast(so[slot], I32)

    def project_ahead(p, src, weights):
        for w, ring in zip(weights, (rq, rk, rv)):
            for c in range(LA // 128):
                t = src[c * 128:(c + 1) * 128, :]
                ring[p, c * 128:(c + 1) * 128, :] = _dot(t, _unpack(w()))

    for cp in head_copies() + unit_copies(0):
        cp.start()

    hbuf[:, pl.ds(0, PAD), :] = jnp.zeros((D // 128, PAD, 128), F32)
    hbuf[:, pl.ds(PAD + S, 3 * PAD + BR), :] = jnp.zeros((D // 128, 3 * PAD + BR, 128), F32)
    xres[pl.ds(S, BR), :] = jnp.zeros((BR, D), F32)
    xn[pl.ds(S, BR), :] = jnp.zeros((BR, D), F32)

    def start_unit(u):
        @pl.when(u < NP)
        def _():
            for cp in unit_copies(u):
                cp.start()

        @pl.when(u + NXH - 1 < S // XB)
        def _():
            xblk_copy(u + NXH - 1).start()

        @pl.when(u == NP)
        def _():
            for cp in b_copies():
                cp.start()

    with SCOPE('head'):
        for cp in head_copies() + unit_copies(0):
            cp.wait()
        start_unit(1)

        def head_rows(b, c):
            x0 = pl.multiple_of(b * XB, XB)
            init_rows(x0, xa, x0)
            return c
        lax.fori_loop(0, NXH, head_rows, 0)
        relayout(0, tmp0)
        start_unit(2)

    def prep_unit(p, cur, nxt):
        @pl.when(p + 1 < NP)
        def _():
            for cp in unit_copies(p + 1):
                cp.wait()

        @pl.when(p + NXH < S // XB)
        def _():
            xblk_copy(p + NXH).wait()

        relayout(jnp.minimum(p + 1, NP - 1), nxt)
        x0 = pl.multiple_of(jnp.minimum(p + NXH, S // XB - 1) * XB, XB)
        init_rows(x0, xn, x0)
        project_ahead(p, xa, [lambda i=i: cur[i] for i in range(3)])
        start_unit(p + 3)

    def prep_two(pp, c):
        prep_unit(2 * pp, tmp0, tmp1)
        prep_unit(2 * pp + 1, tmp1, tmp0)
        return c
    with SCOPE('prep'):
        lax.fori_loop(0, NP // 2, prep_two, 0)

    with SCOPE('bprep'):
        for cp in b_copies():
            cp.wait()
        if B_PACKED:
            for src, dst in ((s1, w1), (s2, w2), (s3, w3), (s4, w4)):
                dst[...] = pltpu.bitcast(src[...], I32)
        else:
            w1, w2, w3, w4 = s1, s2, s3, s4

    def b_rows(jb):
        valid = jb >= 0
        blk = lax.rem(jnp.maximum(jb, 0), NB)
        r0 = pl.multiple_of(jnp.where(valid, blk * BR, S), BR)
        h0 = pl.multiple_of(jnp.where(valid, blk * BR + PAD, S + 3 * PAD), PAD)
        return r0, h0

    def b1_stages(jb):
        r0, h0 = b_rows(jb)
        st = {}

        def s_ln():
            xin = _ln(xres[pl.ds(r0, BR), :])
            xn[pl.ds(r0, BR), :] = xin
            st['t'] = _ln(xin)

        def s_w1():
            hh = _gelu(_dot(st.pop('t'), _unpack(w1[...])))
            for t in range(D // 128):
                hbuf[t, pl.ds(h0, BR), :] = hh[:, t * 128:(t + 1) * 128]
        return [s_ln, s_w1]

    def b2_stages(jb):
        r0, h0 = b_rows(jb)
        st = {}

        def s_w2():
            g = _shift_gather(hbuf, h0, BR)
            x1 = xn[pl.ds(r0, BR), :] + _dot(g, _unpack(w2[...]))
            st['x1'] = x1
            st['u'] = _ln(x1)

        def s_w3():
            st['g'] = _gelu(_dot(st.pop('u'), _unpack(w3[...])))

        def s_w4():
            xo = xres[pl.ds(r0, BR), :] + (st.pop('x1') + _dot(st.pop('g'), _unpack(w4[...])))
            xres[pl.ds(r0, BR), :] = xo
            xn[pl.ds(r0, BR), :] = _ln(xo)
            ob[pl.ds(r0, BR), :] = xo.astype(BF)
        return [s_w2, s_w3, s_w4]

    def out_copy(blk, nblk=1):
        sl = pl.ds(pl.multiple_of(blk * BR, BR), BR * nblk)
        return pltpu.make_async_copy(ob.at[sl, :], o_hbm.at[sl, :], sem_o.at[0])

    def token_rows(j):
        return xn[pl.ds(pl.multiple_of(LA + lax.rem(j, NSEG) * TK, 8), TK), :]

    def step(j, mem, tok, u):
        stages = b1_stages(j - 1) + b2_stages(j - 2)
        hooks = {}
        for t, fn in zip(HOOKS[UNROLL - 1 - u], stages):
            hooks.setdefault(t, []).append(fn)
        s = lax.rem(j, NSEG)
        mem = jnp.where(s == 0, memb[...].astype(F32), mem)
        r0 = pl.multiple_of(s * SEG, SEG)
        n0 = pl.multiple_of(LA + s * TK, 8)
        rd = pl.multiple_of(lax.rem(r0, RING), SEG)
        wr = [pl.multiple_of(lax.rem(n0 + 8 * i, RING), 8) for i in range(TK // 8)]
        h = jnp.concatenate([mem, tok], axis=0)
        o = _a_step(h, rd, wr, wq, wk, wv, wo, rq, rk, rv, hooks)
        xres[pl.ds(r0, SEG), :] = xres[pl.ds(r0, SEG), :] + o[M:, :]
        return o[:M, :]

    OLAG = max(UNROLL, 2)

    def iteration(jj, mem):
        j0 = jj * UNROLL

        @pl.when(j0 == NSEG)
        def _():
            lax.fori_loop(0, NP, lambda p, c: (project_ahead(
                p, xn, [lambda w=w: w[p] for w in (wq, wk, wv)]), c)[1], 0, unroll=PRE_UNROLL)

        toks = [token_rows(j0 + u) for u in range(UNROLL)]
        for u in range(UNROLL):
            mem = step(j0 + u, mem, toks[u], u)

        @pl.when(j0 - OLAG >= NB)
        def _():
            out_copy(j0 - OLAG - NB, UNROLL).start()
        return mem

    with SCOPE('main'):
        lax.fori_loop(0, 2 * NSEG // UNROLL, iteration, memb[...].astype(F32))

    with SCOPE('epilogue'):
        last = 2 * NB - 1
        if OLAG > 2:
            out_copy(NB - OLAG, OLAG - 2).start()
        for fn in b1_stages(last) + b2_stages(last - 1):
            fn()
        out_copy(NB - 2).start()
        for fn in b2_stages(last):
            fn()
        out_copy(NB - 1).start()
    pltpu.make_async_copy(ob.at[pl.ds(0, S), :], o_hbm, sem_o.at[0]).wait()


@jax.jit
def _impl(A_x, A_mem0, A_Wq, A_Wk, A_Wv, A_Wo, B_w1, B_w2, B_w3, B_w4):
    x = A_x.reshape(S, D)
    mem0 = A_mem0.reshape(M, D)
    wqt = jnp.transpose(A_Wq, (1, 2, 0)).reshape(H * E, D)
    wkt = jnp.transpose(A_Wk, (1, 2, 0)).reshape(H * E, D)
    wvt = jnp.transpose(A_Wv, (1, 2, 0)).reshape(H * E, D)
    wo = A_Wo.reshape(H * E, D)
    any_spec = pl.BlockSpec(memory_space=pl.ANY)
    scratch = [
        pltpu.VMEM((S, D), BF),
        pltpu.VMEM((M, D), BF),
        pltpu.VMEM((NSL, PW, D), BF),
        pltpu.VMEM((NSL, PW, D), BF),
        pltpu.VMEM((NSL, PW, D), BF),
        pltpu.VMEM((NSL, PW, D), BF),
        pltpu.VMEM((D, D), BF),
        pltpu.VMEM((D, D), BF),
        pltpu.VMEM((D, F), BF),
        pltpu.VMEM((F, D), BF),
        pltpu.VMEM((NP, D // 2, PW), I32),
        pltpu.VMEM((NP, D // 2, PW), I32),
        pltpu.VMEM((NP, D // 2, PW), I32),
        pltpu.VMEM((NP, PW // 2, D), I32),
        pltpu.VMEM((D // 2, D), I32),
        pltpu.VMEM((D // 2, D), I32),
        pltpu.VMEM((D // 2, F), I32),
        pltpu.VMEM((F // 2, D), I32),
        pltpu.VMEM((S + BR, D), F32),
        pltpu.VMEM((S + BR, D), F32),
        pltpu.VMEM((D // 128, S + 4 * PAD + BR, 128), F32),
        pltpu.VMEM((S + BR, D), BF),
        pltpu.VMEM((NP, RING, PW), F32),
        pltpu.VMEM((NP, RING, PW), F32),
        pltpu.VMEM((NP, RING, PW), F32),
        pltpu.VMEM((LA, D), F32),
        pltpu.VMEM((3, D // 2, PW), I32),
        pltpu.VMEM((3, D // 2, PW), I32),
        pltpu.SemaphoreType.DMA((2,)),
        pltpu.SemaphoreType.DMA((5, NP)),
        pltpu.SemaphoreType.DMA((4,)),
        pltpu.SemaphoreType.DMA((1,)),
    ]
    out = pl.pallas_call(
        _kernel,
        out_shape=jax.ShapeDtypeStruct((S, D), BF),
        in_specs=[any_spec] * 10,
        out_specs=any_spec,
        scratch_shapes=scratch,
        compiler_params=pltpu.CompilerParams(vmem_limit_bytes=126 * 1024 * 1024),
    )(x, mem0, wqt, wkt, wvt, wo, B_w1, B_w2, B_w3, B_w4)
    return out.reshape(1, S, D)


def pallas_interleave_layers__memory_aug_recurrent_mem_tr__mixer_s_mlp__prompt_kernel(
    A_x, A_mem0, A_Wq, A_Wk, A_Wv, A_Wo, A_seg_len, B_x, B_w1, B_w2, B_w3, B_w4,
):
    del B_x
    if isinstance(A_seg_len, int):
        assert A_seg_len == SEG
    assert A_x.shape == (1, S, D)
    return _impl(A_x, A_mem0, A_Wq, A_Wk, A_Wv, A_Wo, B_w1, B_w2, B_w3, B_w4)
```

```python
import contextlib

import jax
import jax.numpy as jnp
from jax import lax
import jax.experimental.pallas as pl
import jax.experimental.pallas.tpu as pltpu

BF = jnp.bfloat16
F32 = jnp.float32
I32 = jnp.int32

S, D, H, E, M, SEG, F = 2048, 640, 32, 192, 8, 32, 1536
L = M + SEG
NSEG = S // SEG
NP = H // 2
PW = 2 * E
SCALE = float(E ** -0.5)
EPS = 1e-5
TK = 24
LA = S - NSEG * TK
RING = LA + SEG
BR = SEG
NB = S // BR
PAD = 8
GROUP = D // 4
XB = 128
NSL = 4
LAGS = (2, 4, 6)
HOOKS = ((1, 3, 7, 10, 13),) + ((1, 3, 7, 14, 99),) * 7
PRE_UNROLL = 2
BW0 = 6
NBW = 8
HEAD_START = 0
UNROLL = 2
B_PACKED = True
NO_BOUNDS_CHECKS = True
PROFILE = False


def SCOPE(name):
    return jax.named_scope(name) if PROFILE else contextlib.nullcontext()


def _ln(x):
    m = jnp.mean(x, axis=-1, keepdims=True)
    c = x - m
    v = jnp.mean(c * c, axis=-1, keepdims=True)
    return c * lax.rsqrt(v + EPS)


def _gelu(x):
    k = 0.7978845608028654
    return 0.5 * x * (1.0 + jnp.tanh(k * (x + 0.044715 * (x * x * x))))


def _dot(a, b):
    return jnp.dot(a, b, preferred_element_type=F32)


def _unpack(w):
    return w if w.dtype == BF else pltpu.bitcast(w, BF)


def _a_step(h, rd, wr, wq, wk, wv, wo, rq, rk, rv, hooks):
    lane = lax.broadcasted_iota(I32, (L, 128), 1)
    lo = lane < 64
    col = lax.broadcasted_iota(I32, (L, 2 * L), 1)
    row = lax.broadcasted_iota(I32, (L, 2 * L), 0)
    first = col < L
    key = jnp.where(first, col, col - L)
    allowed = (row < M) | (row >= key)
    zt = jnp.zeros((L, 128), F32)
    q_, k_, v_, p_, o_ = {}, {}, {}, {}, {}
    acc = [None]

    def blockdiag(t):
        t0, t1, t2 = t[:, 0:128], t[:, 128:256], t[:, 256:384]
        top = jnp.concatenate([t0, jnp.where(lo, t1, 0.0), zt], axis=1)
        bot = jnp.concatenate([zt, jnp.where(lo, 0.0, t1), t2], axis=1)
        return jnp.concatenate([top, bot], axis=0).astype(BF)

    def project(w, ring, p):
        y = _dot(h, _unpack(w[p]))
        for i, r in enumerate(wr):
            ring[p, pl.ds(r, 8), :] = y[M + 8 * i:M + 8 * i + 8, :]
        return y[:M, :]

    def qkv(p):
        q_[p] = project(wq, rq, p)
        k_[p] = project(wk, rk, p)
        v_[p] = project(wv, rv, p)

    def full(mem_rows, ring, p):
        return jnp.concatenate([mem_rows, ring[p, pl.ds(rd, SEG), :]], axis=0)

    def load_qk(p):
        q_[p] = full(q_[p], rq, p)
        k_[p] = blockdiag(full(k_[p], rk, p))

    def load_v(p):
        v_[p] = blockdiag(full(v_[p], rv, p))

    def qk(p):
        s = lax.dot_general(q_.pop(p), k_.pop(p), (((1,), (1,)), ((), ())),
                            preferred_element_type=F32)
        s = jnp.where(allowed, s * SCALE, -1e9)
        m1 = jnp.max(jnp.where(first, s, -jnp.inf), axis=1, keepdims=True)
        m2 = jnp.max(jnp.where(first, -jnp.inf, s), axis=1, keepdims=True)
        e = jnp.exp(s - jnp.where(first, m1, m2))
        l1 = jnp.sum(jnp.where(first, e, 0.0), axis=1, keepdims=True)
        l2 = jnp.sum(jnp.where(first, 0.0, e), axis=1, keepdims=True)
        p_[p] = e * pl.reciprocal(jnp.where(first, l1, l2), approx=False)

    def pv(p):
        o_[p] = _dot(p_.pop(p), v_.pop(p))

    def out(p):
        y = _dot(o_.pop(p), _unpack(wo[p]))
        acc[0] = y if acc[0] is None else acc[0] + y

    la, lb, lc = LAGS
    for t in range(NP + lc):
        for fn in hooks.get(t, ()):
            fn()
        if 0 <= t - la < NP:
            load_qk(t - la)
        if 0 <= t - lb < NP:
            load_v(t - lb)
        if t < NP:
            qkv(t)
        if 0 <= t - la < NP:
            qk(t - la)
        if 0 <= t - lb < NP:
            pv(t - lb)
        if 0 <= t - lc < NP:
            out(t - lc)
    for fn in hooks.get(99, ()):
        fn()
    return acc[0]


def _shift_gather(hbuf, r0, rows):
    lane = lax.broadcasted_iota(I32, (rows, 128), 1)
    shifts = (-1, 1, -2, 2)
    tiles = []
    for t in range(D // 128):
        g_lo = (t * 128) // GROUP
        g_hi = (t * 128 + 127) // GROUP
        a = hbuf[t, pl.ds(r0 + shifts[g_lo], rows), :]
        if g_hi != g_lo:
            b = hbuf[t, pl.ds(r0 + shifts[g_hi], rows), :]
            a = jnp.where(lane < (g_hi * GROUP - t * 128), a, b)
        tiles.append(a)
    return jnp.concatenate(tiles, axis=1)


def _kernel(x_hbm, mem_hbm, wq_hbm, wk_hbm, wv_hbm, wo_hbm, w1_hbm, w2_hbm, w3_hbm, w4_hbm,
            o_hbm,
            xb, memb, sq, sk, sv, so, s1, s2, s3, s4,
            wq, wk, wv, wo, w1, w2, w3, w4,
            xres, xn, hbuf, ob, rq, rk, rv, xa, sem_x, sem_w, sem_b, sem_o):
    NXH = LA // XB

    def mem_copy():
        return pltpu.make_async_copy(mem_hbm, memb, sem_x.at[0])

    def w_copy(i, p):
        src, dst = ((wq_hbm, sq), (wk_hbm, sk), (wv_hbm, sv), (wo_hbm, so))[i]
        return pltpu.make_async_copy(src.at[pl.ds(pl.multiple_of(p * PW, PW), PW), :],
                                     dst.at[lax.rem(p, NSL)], sem_w.at[i, p])

    def xblk_copy(b):
        xs = pl.ds(pl.multiple_of(b * XB, XB), XB)
        return pltpu.make_async_copy(x_hbm.at[xs, :], xb.at[xs, :], sem_w.at[4, b])

    def b_copies(k):
        cps = []
        for i, (src, dst) in enumerate(((w1_hbm, s1), (w2_hbm, s2), (w3_hbm, s3), (w4_hbm, s4))):
            n = src.shape[0] // NBW
            sl = pl.ds(pl.multiple_of(k * n, n), n)
            cps.append(pltpu.make_async_copy(src.at[sl, :], dst.at[sl, :], sem_b.at[i]))
        return cps

    def group(p, action):
        act = (lambda cp: cp.start()) if action == 'start' else (lambda cp: cp.wait())

        @pl.when(p < NP)
        def _():
            act(w_copy(2, p))
            act(w_copy(3, p))

        @pl.when(p + 1 < NP)
        def _():
            act(w_copy(0, p + 1))
            act(w_copy(1, p + 1))

        @pl.when(p + NXH < S // XB)
        def _():
            act(xblk_copy(p + NXH))

    def init_rows(x0, ln_dst):
        x = xb[pl.ds(x0, XB), :].astype(F32)
        xres[pl.ds(x0, XB), :] = x
        ln_dst[pl.ds(x0, XB), :] = _ln(x)

    def relayout(i, p):
        src, dst = ((sq, wq), (sk, wk), (sv, wv))[i]
        dst[p] = pltpu.bitcast(src[lax.rem(p, NSL)].T, I32)

    def project_ahead(i, p, src):
        w, ring = ((wq, rq), (wk, rk), (wv, rv))[i]
        for c in range(LA // 128):
            t = src[c * 128:(c + 1) * 128, :]
            ring[p, c * 128:(c + 1) * 128, :] = _dot(t, _unpack(w[p]))

    for b in range(NXH):
        xblk_copy(b).start()
    w_copy(0, 0).start()
    w_copy(1, 0).start()
    mem_copy().start()

    hbuf[:, pl.ds(0, PAD), :] = jnp.zeros((D // 128, PAD, 128), F32)
    hbuf[:, pl.ds(PAD + S, 3 * PAD + BR), :] = jnp.zeros((D // 128, 3 * PAD + BR, 128), F32)
    xres[pl.ds(S, BR), :] = jnp.zeros((BR, D), F32)
    xn[pl.ds(S, BR), :] = jnp.zeros((BR, D), F32)

    with SCOPE('head'):
        def head_rows(b, c):
            xblk_copy(b).wait()

            @pl.when(b == HEAD_START)
            def _():
                group(0, 'start')

            @pl.when(b == NXH - 1)
            def _():
                group(1, 'start')
            init_rows(pl.multiple_of(b * XB, XB), xa)
            return c
        lax.fori_loop(0, NXH, head_rows, 0)
        w_copy(0, 0).wait()
        w_copy(1, 0).wait()
        mem_copy().wait()
        relayout(0, 0)
        project_ahead(0, 0, xa)
        relayout(1, 0)

    def prep_block(p, last=False):
        group(p, 'wait')
        if not last:
            group(p + 2, 'start')

            @pl.when((p >= BW0) & (p < BW0 + NBW))
            def _():
                for cp in b_copies(p - BW0):
                    cp.start()
        relayout(2, p)
        project_ahead(1, p, xa)
        if not last:
            relayout(0, p + 1)
        project_ahead(2, p, xa)
        wo[p] = pltpu.bitcast(so[lax.rem(p, NSL)], I32)
        if not last:
            relayout(1, p + 1)
            init_rows(pl.multiple_of(jnp.minimum(p + NXH, S // XB - 1) * XB, XB), xn)
            project_ahead(0, p + 1, xa)

    with SCOPE('prep'):
        lax.fori_loop(0, NP - 1, lambda p, c: (prep_block(p), c)[1], 0)
        prep_block(NP - 1, last=True)

    with SCOPE('bprep'):
        for i, (src, dst) in enumerate(((w1_hbm, s1), (w2_hbm, s2), (w3_hbm, s3), (w4_hbm, s4))):
            pltpu.make_async_copy(src, dst, sem_b.at[i]).wait()
        if B_PACKED:
            for src, dst in ((s1, w1), (s2, w2), (s3, w3), (s4, w4)):
                dst[...] = pltpu.bitcast(src[...], I32)
        else:
            w1, w2, w3, w4 = s1, s2, s3, s4

    def b_rows(jb):
        valid = jb >= 0
        blk = lax.rem(jnp.maximum(jb, 0), NB)
        r0 = pl.multiple_of(jnp.where(valid, blk * BR, S), BR)
        h0 = pl.multiple_of(jnp.where(valid, blk * BR + PAD, S + 3 * PAD), PAD)
        return r0, h0

    def b1_stages(jb):
        r0, h0 = b_rows(jb)
        st = {}

        def s_ln():
            xin = _ln(xres[pl.ds(r0, BR), :])
            xn[pl.ds(r0, BR), :] = xin
            st['t'] = _ln(xin)

        def s_w1():
            hh = _gelu(_dot(st.pop('t'), _unpack(w1[...])))
            for t in range(D // 128):
                hbuf[t, pl.ds(h0, BR), :] = hh[:, t * 128:(t + 1) * 128]
        return [s_ln, s_w1]

    def b2_stages(jb):
        r0, h0 = b_rows(jb)
        st = {}

        def s_w2():
            g = _shift_gather(hbuf, h0, BR)
            x1 = xn[pl.ds(r0, BR), :] + _dot(g, _unpack(w2[...]))
            st['x1'] = x1
            st['u'] = _ln(x1)

        def s_w3():
            st['g'] = _gelu(_dot(st.pop('u'), _unpack(w3[...])))

        def s_w4():
            xo = xres[pl.ds(r0, BR), :] + (st.pop('x1') + _dot(st.pop('g'), _unpack(w4[...])))
            xres[pl.ds(r0, BR), :] = xo
            xn[pl.ds(r0, BR), :] = _ln(xo)
            ob[pl.ds(r0, BR), :] = xo.astype(BF)
        return [s_w2, s_w3, s_w4]

    def out_copy(blk, nblk=1):
        sl = pl.ds(pl.multiple_of(blk * BR, BR), BR * nblk)
        return pltpu.make_async_copy(ob.at[sl, :], o_hbm.at[sl, :], sem_o.at[0])

    def token_rows(j):
        return xn[pl.ds(pl.multiple_of(LA + lax.rem(j, NSEG) * TK, 8), TK), :]

    def step(j, mem, tok, u):
        stages = b1_stages(j - 1) + b2_stages(j - 2)
        hooks = {}
        for t, fn in zip(HOOKS[UNROLL - 1 - u], stages):
            hooks.setdefault(t, []).append(fn)
        s = lax.rem(j, NSEG)
        mem = jnp.where(s == 0, memb[...].astype(F32), mem)
        r0 = pl.multiple_of(s * SEG, SEG)
        n0 = pl.multiple_of(LA + s * TK, 8)
        rd = pl.multiple_of(lax.rem(r0, RING), SEG)
        wr = [pl.multiple_of(lax.rem(n0 + 8 * i, RING), 8) for i in range(TK // 8)]
        h = jnp.concatenate([mem, tok], axis=0)
        o = _a_step(h, rd, wr, wq, wk, wv, wo, rq, rk, rv, hooks)
        xres[pl.ds(r0, SEG), :] = xres[pl.ds(r0, SEG), :] + o[M:, :]
        return o[:M, :]

    OLAG = max(UNROLL, 2)

    def iteration(jj, mem):
        j0 = jj * UNROLL

        @pl.when(j0 == NSEG)
        def _():
            def body(p, c):
                for i in range(3):
                    project_ahead(i, p, xn)
                return c
            lax.fori_loop(0, NP, body, 0, unroll=PRE_UNROLL)

        toks = [token_rows(j0 + u) for u in range(UNROLL)]
        for u in range(UNROLL):
            mem = step(j0 + u, mem, toks[u], u)

        @pl.when(j0 - OLAG >= NB)
        def _():
            out_copy(j0 - OLAG - NB, UNROLL).start()
        return mem

    with SCOPE('main'):
        lax.fori_loop(0, 2 * NSEG // UNROLL, iteration, memb[...].astype(F32))

    with SCOPE('epilogue'):
        last = 2 * NB - 1
        if OLAG > 2:
            out_copy(NB - OLAG, OLAG - 2).start()
        for fn in b1_stages(last) + b2_stages(last - 1):
            fn()
        out_copy(NB - 2).start()
        for fn in b2_stages(last):
            fn()
        out_copy(NB - 1).start()
    pltpu.make_async_copy(ob.at[pl.ds(0, S), :], o_hbm, sem_o.at[0]).wait()


@jax.jit
def _impl(A_x, A_mem0, A_Wq, A_Wk, A_Wv, A_Wo, B_w1, B_w2, B_w3, B_w4):
    x = A_x.reshape(S, D)
    mem0 = A_mem0.reshape(M, D)
    wqt = jnp.transpose(A_Wq, (1, 2, 0)).reshape(H * E, D)
    wkt = jnp.transpose(A_Wk, (1, 2, 0)).reshape(H * E, D)
    wvt = jnp.transpose(A_Wv, (1, 2, 0)).reshape(H * E, D)
    wo = A_Wo.reshape(H * E, D)
    any_spec = pl.BlockSpec(memory_space=pl.ANY)
    scratch = [
        pltpu.VMEM((S, D), BF),
        pltpu.VMEM((M, D), BF),
        pltpu.VMEM((NSL, PW, D), BF),
        pltpu.VMEM((NSL, PW, D), BF),
        pltpu.VMEM((NSL, PW, D), BF),
        pltpu.VMEM((NSL, PW, D), BF),
        pltpu.VMEM((D, D), BF),
        pltpu.VMEM((D, D), BF),
        pltpu.VMEM((D, F), BF),
        pltpu.VMEM((F, D), BF),
        pltpu.VMEM((NP, D // 2, PW), I32),
        pltpu.VMEM((NP, D // 2, PW), I32),
        pltpu.VMEM((NP, D // 2, PW), I32),
        pltpu.VMEM((NP, PW // 2, D), I32),
        pltpu.VMEM((D // 2, D), I32),
        pltpu.VMEM((D // 2, D), I32),
        pltpu.VMEM((D // 2, F), I32),
        pltpu.VMEM((F // 2, D), I32),
        pltpu.VMEM((S + BR, D), F32),
        pltpu.VMEM((S + BR, D), F32),
        pltpu.VMEM((D // 128, S + 4 * PAD + BR, 128), F32),
        pltpu.VMEM((S + BR, D), BF),
        pltpu.VMEM((NP, RING, PW), F32),
        pltpu.VMEM((NP, RING, PW), F32),
        pltpu.VMEM((NP, RING, PW), F32),
        pltpu.VMEM((LA, D), F32),
        pltpu.SemaphoreType.DMA((1,)),
        pltpu.SemaphoreType.DMA((5, NP)),
        pltpu.SemaphoreType.DMA((4,)),
        pltpu.SemaphoreType.DMA((1,)),
    ]
    out = pl.pallas_call(
        _kernel,
        out_shape=jax.ShapeDtypeStruct((S, D), BF),
        in_specs=[any_spec] * 10,
        out_specs=any_spec,
        scratch_shapes=scratch,
        compiler_params=pltpu.CompilerParams(vmem_limit_bytes=126 * 1024 * 1024,
                                             disable_bounds_checks=NO_BOUNDS_CHECKS),
    )(x, mem0, wqt, wkt, wvt, wo, B_w1, B_w2, B_w3, B_w4)
    return out.reshape(1, S, D)


def pallas_interleave_layers__memory_aug_recurrent_mem_tr__mixer_s_mlp__prompt_kernel(
    A_x, A_mem0, A_Wq, A_Wk, A_Wv, A_Wo, A_seg_len, B_x, B_w1, B_w2, B_w3, B_w4,
):
    del B_x
    if isinstance(A_seg_len, int):
        assert A_seg_len == SEG
    assert A_x.shape == (1, S, D)
    return _impl(A_x, A_mem0, A_Wq, A_Wk, A_Wv, A_Wo, B_w1, B_w2, B_w3, B_w4)
```

```python
import contextlib

import jax
import jax.numpy as jnp
from jax import lax
import jax.experimental.pallas as pl
import jax.experimental.pallas.tpu as pltpu

BF = jnp.bfloat16
F32 = jnp.float32
I32 = jnp.int32

S, D, H, E, M, SEG, F = 2048, 640, 32, 192, 8, 32, 1536
L = M + SEG
NSEG = S // SEG
NP = H // 2
PW = 2 * E
SCALE = float(E ** -0.5)
EPS = 1e-5
TK = 24
LA = S - NSEG * TK
RING = LA + SEG
BR = SEG
NB = S // BR
PAD = 8
GROUP = D // 4
XB = 128
NSL = 4
LAGS = (1, 3, 5)
HOOKS = ((1, 5, 13, 15, 17), (0, 2, 6, 15, 99))
SLOT_ORDER = ('lv', 'v', 'out', 'lqk', 'q', 'k', 'qk', 'pv')
PRE_UNROLL = 2
BW0 = 6
NBW = 8
HEAD_START = 0
UNROLL = 2
B_PACKED = True
NO_BOUNDS_CHECKS = True
PROFILE = False


def SCOPE(name):
    return jax.named_scope(name) if PROFILE else contextlib.nullcontext()


def _ln(x):
    m = jnp.mean(x, axis=-1, keepdims=True)
    c = x - m
    v = jnp.mean(c * c, axis=-1, keepdims=True)
    return c * lax.rsqrt(v + EPS)


def _gelu(x):
    k = 0.7978845608028654
    return 0.5 * x * (1.0 + jnp.tanh(k * (x + 0.044715 * (x * x * x))))


def _dot(a, b):
    return jnp.dot(a, b, preferred_element_type=F32)


def _unpack(w):
    return w if w.dtype == BF else pltpu.bitcast(w, BF)


def _a_step(h, rd, wr, wq, wk, wv, wo, rq, rk, rv, hooks):
    lane = lax.broadcasted_iota(I32, (L, 128), 1)
    lo = lane < 64
    col = lax.broadcasted_iota(I32, (L, 2 * L), 1)
    row = lax.broadcasted_iota(I32, (L, 2 * L), 0)
    first = col < L
    key = jnp.where(first, col, col - L)
    allowed = (row < M) | (row >= key)
    zt = jnp.zeros((L, 128), F32)
    q_, k_, v_, p_, o_ = {}, {}, {}, {}, {}
    acc = [None]

    def blockdiag(t):
        t0, t1, t2 = t[:, 0:128], t[:, 128:256], t[:, 256:384]
        top = jnp.concatenate([t0, jnp.where(lo, t1, 0.0), zt], axis=1)
        bot = jnp.concatenate([zt, jnp.where(lo, 0.0, t1), t2], axis=1)
        return jnp.concatenate([top, bot], axis=0).astype(BF)

    def project(w, ring, p):
        y = _dot(h, _unpack(w[p]))
        for i, r in enumerate(wr):
            ring[p, pl.ds(r, 8), :] = y[M + 8 * i:M + 8 * i + 8, :]
        return y[:M, :]

    def proj_q(p):
        q_[p] = project(wq, rq, p)

    def proj_k(p):
        k_[p] = project(wk, rk, p)

    def proj_v(p):
        v_[p] = project(wv, rv, p)

    def full(mem_rows, ring, p):
        return jnp.concatenate([mem_rows, ring[p, pl.ds(rd, SEG), :]], axis=0)

    def load_qk(p):
        q_[p] = full(q_[p], rq, p)
        k_[p] = blockdiag(full(k_[p], rk, p))

    def load_v(p):
        v_[p] = blockdiag(full(v_[p], rv, p))

    def qk(p):
        s = lax.dot_general(q_.pop(p), k_.pop(p), (((1,), (1,)), ((), ())),
                            preferred_element_type=F32)
        s = jnp.where(allowed, s * SCALE, -1e9)
        m1 = jnp.max(jnp.where(first, s, -jnp.inf), axis=1, keepdims=True)
        m2 = jnp.max(jnp.where(first, -jnp.inf, s), axis=1, keepdims=True)
        e = jnp.exp(s - jnp.where(first, m1, m2))
        l1 = jnp.sum(jnp.where(first, e, 0.0), axis=1, keepdims=True)
        l2 = jnp.sum(jnp.where(first, 0.0, e), axis=1, keepdims=True)
        p_[p] = e * pl.reciprocal(jnp.where(first, l1, l2), approx=False)

    def pv(p):
        o_[p] = _dot(p_.pop(p), v_.pop(p))

    def out(p):
        y = _dot(o_.pop(p), _unpack(wo[p]))
        acc[0] = y if acc[0] is None else acc[0] + y

    la, lb, lc = LAGS
    for t in range(NP + lc):
        for fn in hooks.get(t, ()):
            fn()
        for name in SLOT_ORDER:
            fn, lag = dict(q=(proj_q, 0), k=(proj_k, 0), v=(proj_v, 0), lqk=(load_qk, la),
                           lv=(load_v, lb), qk=(qk, la), pv=(pv, lb), out=(out, lc))[name]
            if 0 <= t - lag < NP:
                fn(t - lag)
    for fn in hooks.get(99, ()):
        fn()
    return acc[0]


def _shift_gather(hbuf, r0, rows):
    lane = lax.broadcasted_iota(I32, (rows, 128), 1)
    shifts = (-1, 1, -2, 2)
    tiles = []
    for t in range(D // 128):
        g_lo = (t * 128) // GROUP
        g_hi = (t * 128 + 127) // GROUP
        a = hbuf[t, pl.ds(r0 + shifts[g_lo], rows), :]
        if g_hi != g_lo:
            b = hbuf[t, pl.ds(r0 + shifts[g_hi], rows), :]
            a = jnp.where(lane < (g_hi * GROUP - t * 128), a, b)
        tiles.append(a)
    return jnp.concatenate(tiles, axis=1)


def _kernel(x_hbm, mem_hbm, wq_hbm, wk_hbm, wv_hbm, wo_hbm, w1_hbm, w2_hbm, w3_hbm, w4_hbm,
            o_hbm,
            xb, memb, sq, sk, sv, so, s1, s2, s3, s4,
            wq, wk, wv, wo, w1, w2, w3, w4,
            xres, xn, hbuf, ob, rq, rk, rv, xa, sem_x, sem_w, sem_b, sem_o):
    NXH = LA // XB

    def mem_copy():
        return pltpu.make_async_copy(mem_hbm, memb, sem_x.at[0])

    def w_copy(i, p):
        src, dst = ((wq_hbm, sq), (wk_hbm, sk), (wv_hbm, sv), (wo_hbm, so))[i]
        return pltpu.make_async_copy(src.at[pl.ds(pl.multiple_of(p * PW, PW), PW), :],
                                     dst.at[lax.rem(p, NSL)], sem_w.at[i, p])

    def xblk_copy(b):
        xs = pl.ds(pl.multiple_of(b * XB, XB), XB)
        return pltpu.make_async_copy(x_hbm.at[xs, :], xb.at[xs, :], sem_w.at[4, b])

    def b_copies(k):
        cps = []
        for i, (src, dst) in enumerate(((w1_hbm, s1), (w2_hbm, s2), (w3_hbm, s3), (w4_hbm, s4))):
            n = src.shape[0] // NBW
            sl = pl.ds(pl.multiple_of(k * n, n), n)
            cps.append(pltpu.make_async_copy(src.at[sl, :], dst.at[sl, :], sem_b.at[i]))
        return cps

    def group(p, action):
        act = (lambda cp: cp.start()) if action == 'start' else (lambda cp: cp.wait())

        @pl.when(p < NP)
        def _():
            act(w_copy(2, p))
            act(w_copy(3, p))

        @pl.when(p + 1 < NP)
        def _():
            act(w_copy(0, p + 1))
            act(w_copy(1, p + 1))

        @pl.when(p + NXH < S // XB)
        def _():
            act(xblk_copy(p + NXH))

    def init_rows(x0, ln_dst):
        x = xb[pl.ds(x0, XB), :].astype(F32)
        xres[pl.ds(x0, XB), :] = x
        ln_dst[pl.ds(x0, XB), :] = _ln(x)

    def relayout(i, p):
        src, dst = ((sq, wq), (sk, wk), (sv, wv))[i]
        dst[p] = pltpu.bitcast(src[lax.rem(p, NSL)].T, I32)

    def project_ahead(i, p, src):
        w, ring = ((wq, rq), (wk, rk), (wv, rv))[i]
        for c in range(LA // 128):
            t = src[c * 128:(c + 1) * 128, :]
            ring[p, c * 128:(c + 1) * 128, :] = _dot(t, _unpack(w[p]))

    for b in range(NXH):
        xblk_copy(b).start()
    w_copy(0, 0).start()
    w_copy(1, 0).start()
    mem_copy().start()

    hbuf[:, pl.ds(0, PAD), :] = jnp.zeros((D // 128, PAD, 128), F32)
    hbuf[:, pl.ds(PAD + S, 3 * PAD + BR), :] = jnp.zeros((D // 128, 3 * PAD + BR, 128), F32)
    xres[pl.ds(S, BR), :] = jnp.zeros((BR, D), F32)
    xn[pl.ds(S, BR), :] = jnp.zeros((BR, D), F32)

    with SCOPE('head'):
        def head_rows(b, c):
            xblk_copy(b).wait()

            @pl.when(b == HEAD_START)
            def _():
                group(0, 'start')

            @pl.when(b == NXH - 1)
            def _():
                group(1, 'start')
            init_rows(pl.multiple_of(b * XB, XB), xa)
            return c
        lax.fori_loop(0, NXH, head_rows, 0)
        w_copy(0, 0).wait()
        w_copy(1, 0).wait()
        mem_copy().wait()
        relayout(0, 0)
        project_ahead(0, 0, xa)
        relayout(1, 0)

    def prep_block(p, last=False):
        group(p, 'wait')
        if not last:
            group(p + 2, 'start')

            @pl.when((p >= BW0) & (p < BW0 + NBW))
            def _():
                for cp in b_copies(p - BW0):
                    cp.start()
        relayout(2, p)
        project_ahead(1, p, xa)
        if not last:
            relayout(0, p + 1)
        project_ahead(2, p, xa)
        wo[p] = pltpu.bitcast(so[lax.rem(p, NSL)], I32)
        if not last:
            relayout(1, p + 1)
            init_rows(pl.multiple_of(jnp.minimum(p + NXH, S // XB - 1) * XB, XB), xn)
            project_ahead(0, p + 1, xa)

    with SCOPE('prep'):
        lax.fori_loop(0, NP - 1, lambda p, c: (prep_block(p), c)[1], 0)
        prep_block(NP - 1, last=True)

    with SCOPE('bprep'):
        for i, (src, dst) in enumerate(((w1_hbm, s1), (w2_hbm, s2), (w3_hbm, s3), (w4_hbm, s4))):
            pltpu.make_async_copy(src, dst, sem_b.at[i]).wait()
        if B_PACKED:
            for src, dst in ((s1, w1), (s2, w2), (s3, w3), (s4, w4)):
                dst[...] = pltpu.bitcast(src[...], I32)
        else:
            w1, w2, w3, w4 = s1, s2, s3, s4

    def b_rows(jb):
        valid = jb >= 0
        blk = lax.rem(jnp.maximum(jb, 0), NB)
        r0 = pl.multiple_of(jnp.where(valid, blk * BR, S), BR)
        h0 = pl.multiple_of(jnp.where(valid, blk * BR + PAD, S + 3 * PAD), PAD)
        return r0, h0

    def b1_stages(jb):
        r0, h0 = b_rows(jb)
        st = {}

        def s_ln():
            xin = _ln(xres[pl.ds(r0, BR), :])
            xn[pl.ds(r0, BR), :] = xin
            st['t'] = _ln(xin)

        def s_w1():
            hh = _gelu(_dot(st.pop('t'), _unpack(w1[...])))
            for t in range(D // 128):
                hbuf[t, pl.ds(h0, BR), :] = hh[:, t * 128:(t + 1) * 128]
        return [s_ln, s_w1]

    def b2_stages(jb):
        r0, h0 = b_rows(jb)
        st = {}

        def s_w2():
            g = _shift_gather(hbuf, h0, BR)
            x1 = xn[pl.ds(r0, BR), :] + _dot(g, _unpack(w2[...]))
            st['x1'] = x1
            st['u'] = _ln(x1)

        def s_w3():
            st['g'] = _gelu(_dot(st.pop('u'), _unpack(w3[...])))

        def s_w4():
            xo = xres[pl.ds(r0, BR), :] + (st.pop('x1') + _dot(st.pop('g'), _unpack(w4[...])))
            xres[pl.ds(r0, BR), :] = xo
            xn[pl.ds(r0, BR), :] = _ln(xo)
            ob[pl.ds(r0, BR), :] = xo.astype(BF)
        return [s_w2, s_w3, s_w4]

    def out_copy(blk, nblk=1):
        sl = pl.ds(pl.multiple_of(blk * BR, BR), BR * nblk)
        return pltpu.make_async_copy(ob.at[sl, :], o_hbm.at[sl, :], sem_o.at[0])

    def token_rows(j):
        return xn[pl.ds(pl.multiple_of(LA + lax.rem(j, NSEG) * TK, 8), TK), :]

    def step(j, mem, tok, u):
        stages = b1_stages(j - 1) + b2_stages(j - 2)
        hooks = {}
        for t, fn in zip(HOOKS[UNROLL - 1 - u], stages):
            hooks.setdefault(t, []).append(fn)
        s = lax.rem(j, NSEG)
        mem = jnp.where(s == 0, memb[...].astype(F32), mem)
        r0 = pl.multiple_of(s * SEG, SEG)
        n0 = pl.multiple_of(LA + s * TK, 8)
        rd = pl.multiple_of(lax.rem(r0, RING), SEG)
        wr = [pl.multiple_of(lax.rem(n0 + 8 * i, RING), 8) for i in range(TK // 8)]
        h = jnp.concatenate([mem, tok], axis=0)
        o = _a_step(h, rd, wr, wq, wk, wv, wo, rq, rk, rv, hooks)
        xres[pl.ds(r0, SEG), :] = xres[pl.ds(r0, SEG), :] + o[M:, :]
        return o[:M, :]

    OLAG = max(UNROLL, 2)

    def iteration(jj, mem):
        j0 = jj * UNROLL

        @pl.when(j0 == NSEG)
        def _():
            def body(p, c):
                for i in range(3):
                    project_ahead(i, p, xn)
                return c
            lax.fori_loop(0, NP, body, 0, unroll=PRE_UNROLL)

        toks = [token_rows(j0 + u) for u in range(UNROLL)]
        for u in range(UNROLL):
            mem = step(j0 + u, mem, toks[u], u)

        @pl.when(j0 - OLAG >= NB)
        def _():
            out_copy(j0 - OLAG - NB, UNROLL).start()
        return mem

    with SCOPE('main'):
        lax.fori_loop(0, 2 * NSEG // UNROLL, iteration, memb[...].astype(F32))

    with SCOPE('epilogue'):
        last = 2 * NB - 1
        if OLAG > 2:
            out_copy(NB - OLAG, OLAG - 2).start()
        for fn in b1_stages(last) + b2_stages(last - 1):
            fn()
        out_copy(NB - 2).start()
        for fn in b2_stages(last):
            fn()
        out_copy(NB - 1).start()
    pltpu.make_async_copy(ob.at[pl.ds(0, S), :], o_hbm, sem_o.at[0]).wait()


@jax.jit
def _impl(A_x, A_mem0, A_Wq, A_Wk, A_Wv, A_Wo, B_w1, B_w2, B_w3, B_w4):
    x = A_x.reshape(S, D)
    mem0 = A_mem0.reshape(M, D)
    wqt = jnp.transpose(A_Wq, (1, 2, 0)).reshape(H * E, D)
    wkt = jnp.transpose(A_Wk, (1, 2, 0)).reshape(H * E, D)
    wvt = jnp.transpose(A_Wv, (1, 2, 0)).reshape(H * E, D)
    wo = A_Wo.reshape(H * E, D)
    any_spec = pl.BlockSpec(memory_space=pl.ANY)
    scratch = [
        pltpu.VMEM((S, D), BF),
        pltpu.VMEM((M, D), BF),
        pltpu.VMEM((NSL, PW, D), BF),
        pltpu.VMEM((NSL, PW, D), BF),
        pltpu.VMEM((NSL, PW, D), BF),
        pltpu.VMEM((NSL, PW, D), BF),
        pltpu.VMEM((D, D), BF),
        pltpu.VMEM((D, D), BF),
        pltpu.VMEM((D, F), BF),
        pltpu.VMEM((F, D), BF),
        pltpu.VMEM((NP, D // 2, PW), I32),
        pltpu.VMEM((NP, D // 2, PW), I32),
        pltpu.VMEM((NP, D // 2, PW), I32),
        pltpu.VMEM((NP, PW // 2, D), I32),
        pltpu.VMEM((D // 2, D), I32),
        pltpu.VMEM((D // 2, D), I32),
        pltpu.VMEM((D // 2, F), I32),
        pltpu.VMEM((F // 2, D), I32),
        pltpu.VMEM((S + BR, D), F32),
        pltpu.VMEM((S + BR, D), F32),
        pltpu.VMEM((D // 128, S + 4 * PAD + BR, 128), F32),
        pltpu.VMEM((S + BR, D), BF),
        pltpu.VMEM((NP, RING, PW), F32),
        pltpu.VMEM((NP, RING, PW), F32),
        pltpu.VMEM((NP, RING, PW), F32),
        pltpu.VMEM((LA, D), F32),
        pltpu.SemaphoreType.DMA((1,)),
        pltpu.SemaphoreType.DMA((5, NP)),
        pltpu.SemaphoreType.DMA((4,)),
        pltpu.SemaphoreType.DMA((1,)),
    ]
    out = pl.pallas_call(
        _kernel,
        out_shape=jax.ShapeDtypeStruct((S, D), BF),
        in_specs=[any_spec] * 10,
        out_specs=any_spec,
        scratch_shapes=scratch,
        compiler_params=pltpu.CompilerParams(vmem_limit_bytes=126 * 1024 * 1024,
                                             disable_bounds_checks=NO_BOUNDS_CHECKS),
    )(x, mem0, wqt, wkt, wvt, wo, B_w1, B_w2, B_w3, B_w4)
    return out.reshape(1, S, D)


def pallas_interleave_layers__memory_aug_recurrent_mem_tr__mixer_s_mlp__prompt_kernel(
    A_x, A_mem0, A_Wq, A_Wk, A_Wv, A_Wo, A_seg_len, B_x, B_w1, B_w2, B_w3, B_w4,
):
    del B_x
    if isinstance(A_seg_len, int):
        assert A_seg_len == SEG
    assert A_x.shape == (1, S, D)
    return _impl(A_x, A_mem0, A_Wq, A_Wk, A_Wv, A_Wo, B_w1, B_w2, B_w3, B_w4)
```

```python
import contextlib

import jax
import jax.numpy as jnp
from jax import lax
import jax.experimental.pallas as pl
import jax.experimental.pallas.tpu as pltpu

BF = jnp.bfloat16
F32 = jnp.float32
I32 = jnp.int32

S, D, H, E, M, SEG, F = 2048, 640, 32, 192, 8, 32, 1536
L = M + SEG
NSEG = S // SEG
NP = H // 2
PW = 2 * E
SCALE = float(E ** -0.5)
EPS = 1e-5
TK = 24
LA = S - NSEG * TK
RING = LA + SEG
BR = SEG
NB = S // BR
PAD = 8
GROUP = D // 4
XB = 128
NSL = 4
LAGS = (1, 3, 5)
HOOKS = ((1, 5, 11, 15, 18), (1, 2, 6, 15, 99))
SLOT_ORDER = ('lv', 'v', 'out', 'lqk', 'q', 'k', 'qk', 'pv')
PRE_UNROLL = 4
BW0 = 6
NBW = 8
HEAD_PLAN = dict(q0='t0', k0='b0', g0a='b0', g0b='w', g1a='w', g1b='end')
UNROLL = 2
NO_BOUNDS_CHECKS = True
PROFILE = False


def SCOPE(name):
    return jax.named_scope(name) if PROFILE else contextlib.nullcontext()


def _ln(x):
    m = jnp.mean(x, axis=-1, keepdims=True)
    c = x - m
    v = jnp.mean(c * c, axis=-1, keepdims=True)
    return c * lax.rsqrt(v + EPS)


def _gelu(x):
    k = 0.7978845608028654
    return 0.5 * x * (1.0 + jnp.tanh(k * (x + 0.044715 * (x * x * x))))


def _dot(a, b):
    return jnp.dot(a, b, preferred_element_type=F32)


def _unpack(w):
    return pltpu.bitcast(w, BF)


def _a_step(h, rd, wr, wq, wk, wv, wo, rq, rk, rv, hooks):
    lane = lax.broadcasted_iota(I32, (L, 128), 1)
    lo = lane < 64
    col = lax.broadcasted_iota(I32, (L, 2 * L), 1)
    row = lax.broadcasted_iota(I32, (L, 2 * L), 0)
    first = col < L
    key = jnp.where(first, col, col - L)
    allowed = (row < M) | (row >= key)
    zt = jnp.zeros((L, 128), F32)
    q_, k_, v_, p_, o_ = {}, {}, {}, {}, {}
    acc = [None]

    def blockdiag(t):
        t0, t1, t2 = t[:, 0:128], t[:, 128:256], t[:, 256:384]
        top = jnp.concatenate([t0, jnp.where(lo, t1, 0.0), zt], axis=1)
        bot = jnp.concatenate([zt, jnp.where(lo, 0.0, t1), t2], axis=1)
        return jnp.concatenate([top, bot], axis=0).astype(BF)

    def project(w, ring, p):
        y = _dot(h, _unpack(w[p]))
        for i, r in enumerate(wr):
            ring[p, pl.ds(r, 8), :] = y[M + 8 * i:M + 8 * i + 8, :]
        return y[:M, :]

    def proj_q(p):
        q_[p] = project(wq, rq, p)

    def proj_k(p):
        k_[p] = project(wk, rk, p)

    def proj_v(p):
        v_[p] = project(wv, rv, p)

    def full(mem_rows, ring, p):
        return jnp.concatenate([mem_rows, ring[p, pl.ds(rd, SEG), :]], axis=0)

    def load_qk(p):
        q_[p] = full(q_[p], rq, p)
        k_[p] = blockdiag(full(k_[p], rk, p))

    def load_v(p):
        v_[p] = blockdiag(full(v_[p], rv, p))

    def qk(p):
        s = lax.dot_general(q_.pop(p), k_.pop(p), (((1,), (1,)), ((), ())),
                            preferred_element_type=F32)
        s = jnp.where(allowed, s * SCALE, -1e9)
        m1 = jnp.max(jnp.where(first, s, -jnp.inf), axis=1, keepdims=True)
        m2 = jnp.max(jnp.where(first, -jnp.inf, s), axis=1, keepdims=True)
        e = jnp.exp(s - jnp.where(first, m1, m2))
        l1 = jnp.sum(jnp.where(first, e, 0.0), axis=1, keepdims=True)
        l2 = jnp.sum(jnp.where(first, 0.0, e), axis=1, keepdims=True)
        p_[p] = e * pl.reciprocal(jnp.where(first, l1, l2), approx=False)

    def pv(p):
        o_[p] = _dot(p_.pop(p), v_.pop(p))

    def out(p):
        y = _dot(o_.pop(p), _unpack(wo[p]))
        acc[0] = y if acc[0] is None else acc[0] + y

    la, lb, lc = LAGS
    for t in range(NP + lc):
        for fn in hooks.get(t, ()):
            fn()
        for name in SLOT_ORDER:
            fn, lag = dict(q=(proj_q, 0), k=(proj_k, 0), v=(proj_v, 0), lqk=(load_qk, la),
                           lv=(load_v, lb), qk=(qk, la), pv=(pv, lb), out=(out, lc))[name]
            if 0 <= t - lag < NP:
                fn(t - lag)
    for fn in hooks.get(99, ()):
        fn()
    return acc[0]


def _shift_gather(hbuf, r0, rows):
    lane = lax.broadcasted_iota(I32, (rows, 128), 1)
    shifts = (-1, 1, -2, 2)
    tiles = []
    for t in range(D // 128):
        g_lo = (t * 128) // GROUP
        g_hi = (t * 128 + 127) // GROUP
        a = hbuf[t, pl.ds(r0 + shifts[g_lo], rows), :]
        if g_hi != g_lo:
            b = hbuf[t, pl.ds(r0 + shifts[g_hi], rows), :]
            a = jnp.where(lane < (g_hi * GROUP - t * 128), a, b)
        tiles.append(a)
    return jnp.concatenate(tiles, axis=1)


def _kernel(x_hbm, mem_hbm, wq_hbm, wk_hbm, wv_hbm, wo_hbm, w1_hbm, w2_hbm, w3_hbm, w4_hbm,
            o_hbm,
            xb, memb, sq, sk, sv, so, s1, s2, s3, s4,
            wq, wk, wv, wo, w1, w2, w3, w4,
            xres, xn, hbuf, ob, rq, rk, rv, xa, sem_x, sem_w, sem_b, sem_o):
    NXH = LA // XB

    def mem_copy():
        return pltpu.make_async_copy(mem_hbm, memb, sem_x.at[0])

    def w_copy(i, p):
        src, dst = ((wq_hbm, sq), (wk_hbm, sk), (wv_hbm, sv), (wo_hbm, so))[i]
        return pltpu.make_async_copy(src.at[pl.ds(pl.multiple_of(p * PW, PW), PW), :],
                                     dst.at[lax.rem(p, NSL)], sem_w.at[i, p])

    def xblk_copy(b):
        xs = pl.ds(pl.multiple_of(b * XB, XB), XB)
        return pltpu.make_async_copy(x_hbm.at[xs, :], xb.at[xs, :], sem_w.at[4, b])

    def b_copies(k):
        cps = []
        for i, (src, dst) in enumerate(((w1_hbm, s1), (w2_hbm, s2), (w3_hbm, s3), (w4_hbm, s4))):
            n = src.shape[0] // NBW
            sl = pl.ds(pl.multiple_of(k * n, n), n)
            cps.append(pltpu.make_async_copy(src.at[sl, :], dst.at[sl, :], sem_b.at[i]))
        return cps

    def group(p, action, part=None):
        act = (lambda cp: cp.start()) if action == 'start' else (lambda cp: cp.wait())
        if part in (None, 0):
            @pl.when(p < NP)
            def _():
                act(w_copy(2, p))
        if part in (None, 1):
            @pl.when(p < NP)
            def _():
                act(w_copy(3, p))

            @pl.when(p + 1 < NP)
            def _():
                act(w_copy(0, p + 1))
                act(w_copy(1, p + 1))

            @pl.when(p + NXH < S // XB)
            def _():
                act(xblk_copy(p + NXH))

    def init_rows(x0, ln_dst):
        x = xb[pl.ds(x0, XB), :].astype(F32)
        xres[pl.ds(x0, XB), :] = x
        ln_dst[pl.ds(x0, XB), :] = _ln(x)

    def relayout(i, p):
        src, dst = ((sq, wq), (sk, wk), (sv, wv))[i]
        dst[p] = pltpu.bitcast(src[lax.rem(p, NSL)].T, I32)

    def project_ahead(i, p, src):
        w, ring = ((wq, rq), (wk, rk), (wv, rv))[i]
        for c in range(LA // 128):
            t = src[c * 128:(c + 1) * 128, :]
            ring[p, c * 128:(c + 1) * 128, :] = _dot(t, _unpack(w[p]))

    def trigger(name):
        for what, when in HEAD_PLAN.items():
            if when == name:
                dict(q0=lambda: w_copy(0, 0).start(), k0=lambda: w_copy(1, 0).start(),
                     g0a=lambda: group(0, 'start', 0), g0b=lambda: group(0, 'start', 1),
                     g1a=lambda: group(1, 'start', 0), g1b=lambda: group(1, 'start', 1))[what]()

    trigger('t0')
    for b in range(NXH):
        xblk_copy(b).start()
    mem_copy().start()
    trigger('t1')

    hbuf[:, pl.ds(0, PAD), :] = jnp.zeros((D // 128, PAD, 128), F32)
    hbuf[:, pl.ds(PAD + S, 3 * PAD + BR), :] = jnp.zeros((D // 128, 3 * PAD + BR, 128), F32)
    xres[pl.ds(S, BR), :] = jnp.zeros((BR, D), F32)
    xn[pl.ds(S, BR), :] = jnp.zeros((BR, D), F32)

    with SCOPE('head'):
        for b in range(NXH):
            xblk_copy(b).wait()
            trigger('b%d' % b)
        w_copy(0, 0).wait()
        mem_copy().wait()
        trigger('w')
        for b in range(NXH):
            init_rows(b * XB, xa)
        relayout(0, 0)
        project_ahead(0, 0, xa)
        w_copy(1, 0).wait()
        relayout(1, 0)
        trigger('end')

    def prep_block(p):
        group(p, 'wait', 0)
        group(p + 2, 'start')

        @pl.when((p >= BW0) & (p < BW0 + NBW))
        def _():
            for cp in b_copies(p - BW0):
                cp.start()
        relayout(2, p)
        project_ahead(1, p, xa)
        group(p, 'wait', 1)
        relayout(0, p + 1)
        project_ahead(2, p, xa)
        wo[p] = pltpu.bitcast(so[lax.rem(p, NSL)], I32)
        relayout(1, p + 1)
        init_rows(pl.multiple_of(jnp.minimum(p + NXH, S // XB - 1) * XB, XB), xn)
        project_ahead(0, p + 1, xa)

    def prep_last():
        p = NP - 1
        group(p, 'wait')
        for i, (src, dst) in enumerate(((w1_hbm, s1), (w2_hbm, s2), (w3_hbm, s3), (w4_hbm, s4))):
            pltpu.make_async_copy(src, dst, sem_b.at[i]).wait()
        relayout(2, p)
        for src, dst in ((s1, w1), (s2, w2), (s3, w3), (s4, w4)):
            dst[...] = pltpu.bitcast(src[...], I32)
        project_ahead(1, p, xa)
        project_ahead(2, p, xa)
        wo[p] = pltpu.bitcast(so[lax.rem(p, NSL)], I32)

    with SCOPE('prep'):
        lax.fori_loop(0, NP - 1, lambda p, c: (prep_block(p), c)[1], 0)
        prep_last()

    def b_rows(jb):
        valid = jb >= 0
        blk = lax.rem(jnp.maximum(jb, 0), NB)
        r0 = pl.multiple_of(jnp.where(valid, blk * BR, S), BR)
        h0 = pl.multiple_of(jnp.where(valid, blk * BR + PAD, S + 3 * PAD), PAD)
        return r0, h0

    def b1_stages(jb):
        r0, h0 = b_rows(jb)
        st = {}

        def s_ln():
            xin = _ln(xres[pl.ds(r0, BR), :])
            xn[pl.ds(r0, BR), :] = xin
            st['t'] = _ln(xin)

        def s_w1():
            hh = _gelu(_dot(st.pop('t'), _unpack(w1[...])))
            for t in range(D // 128):
                hbuf[t, pl.ds(h0, BR), :] = hh[:, t * 128:(t + 1) * 128]
        return [s_ln, s_w1]

    def b2_stages(jb, BR=BR):
        r0, h0 = b_rows(jb)
        st = {}

        def s_w2():
            g = _shift_gather(hbuf, h0, BR)
            x1 = xn[pl.ds(r0, BR), :] + _dot(g, _unpack(w2[...]))
            st['x1'] = x1
            st['u'] = _ln(x1)

        def s_w3():
            st['g'] = _gelu(_dot(st.pop('u'), _unpack(w3[...])))

        def s_w4():
            xo = xres[pl.ds(r0, BR), :] + (st.pop('x1') + _dot(st.pop('g'), _unpack(w4[...])))
            xres[pl.ds(r0, BR), :] = xo
            xn[pl.ds(r0, BR), :] = _ln(xo)
            ob[pl.ds(r0, BR), :] = xo.astype(BF)
        return [s_w2, s_w3, s_w4]

    def out_copy(blk, nblk=1):
        sl = pl.ds(pl.multiple_of(blk * BR, BR), BR * nblk)
        return pltpu.make_async_copy(ob.at[sl, :], o_hbm.at[sl, :], sem_o.at[0])

    def token_rows(j):
        return xn[pl.ds(pl.multiple_of(LA + lax.rem(j, NSEG) * TK, 8), TK), :]

    def step(j, mem, tok, u):
        stages = b1_stages(j - 1) + b2_stages(j - 2)
        hooks = {}
        for t, fn in zip(HOOKS[UNROLL - 1 - u], stages):
            hooks.setdefault(t, []).append(fn)
        s = lax.rem(j, NSEG)
        mem = jnp.where(s == 0, memb[...].astype(F32), mem)
        r0 = pl.multiple_of(s * SEG, SEG)
        n0 = pl.multiple_of(LA + s * TK, 8)
        rd = pl.multiple_of(lax.rem(r0, RING), SEG)
        wr = [pl.multiple_of(lax.rem(n0 + 8 * i, RING), 8) for i in range(TK // 8)]
        h = jnp.concatenate([mem, tok], axis=0)
        o = _a_step(h, rd, wr, wq, wk, wv, wo, rq, rk, rv, hooks)
        xres[pl.ds(r0, SEG), :] = xres[pl.ds(r0, SEG), :] + o[M:, :]
        return o[:M, :]

    OLAG = max(UNROLL, 2)

    def iteration(jj, mem):
        j0 = jj * UNROLL

        @pl.when(j0 == NSEG)
        def _():
            def body(p, c):
                for i in range(3):
                    project_ahead(i, p, xn)
                return c
            lax.fori_loop(0, NP, body, 0, unroll=PRE_UNROLL)

        toks = [token_rows(j0 + u) for u in range(UNROLL)]
        for u in range(UNROLL):
            mem = step(j0 + u, mem, toks[u], u)

        @pl.when(j0 - OLAG >= NB)
        def _():
            out_copy(j0 - OLAG - NB, UNROLL).start()
        return mem

    with SCOPE('main'):
        lax.fori_loop(0, 2 * NSEG // UNROLL, iteration, memb[...].astype(F32))

    with SCOPE('epilogue'):
        last = 2 * NB - 1
        if OLAG > 2:
            out_copy(NB - OLAG, OLAG - 2).start()
        for fn in b1_stages(last) + b2_stages(last - 1, 2 * BR):
            fn()
        out_copy(NB - 2, 2).start()
    pltpu.make_async_copy(ob.at[pl.ds(0, S), :], o_hbm, sem_o.at[0]).wait()


@jax.jit
def _impl(A_x, A_mem0, A_Wq, A_Wk, A_Wv, A_Wo, B_w1, B_w2, B_w3, B_w4):
    x = A_x.reshape(S, D)
    mem0 = A_mem0.reshape(M, D)
    wqt = jnp.transpose(A_Wq, (1, 2, 0)).reshape(H * E, D)
    wkt = jnp.transpose(A_Wk, (1, 2, 0)).reshape(H * E, D)
    wvt = jnp.transpose(A_Wv, (1, 2, 0)).reshape(H * E, D)
    wo = A_Wo.reshape(H * E, D)
    any_spec = pl.BlockSpec(memory_space=pl.ANY)
    scratch = [
        pltpu.VMEM((S, D), BF),
        pltpu.VMEM((M, D), BF),
        pltpu.VMEM((NSL, PW, D), BF),
        pltpu.VMEM((NSL, PW, D), BF),
        pltpu.VMEM((NSL, PW, D), BF),
        pltpu.VMEM((NSL, PW, D), BF),
        pltpu.VMEM((D, D), BF),
        pltpu.VMEM((D, D), BF),
        pltpu.VMEM((D, F), BF),
        pltpu.VMEM((F, D), BF),
        pltpu.VMEM((NP, D // 2, PW), I32),
        pltpu.VMEM((NP, D // 2, PW), I32),
        pltpu.VMEM((NP, D // 2, PW), I32),
        pltpu.VMEM((NP, PW // 2, D), I32),
        pltpu.VMEM((D // 2, D), I32),
        pltpu.VMEM((D // 2, D), I32),
        pltpu.VMEM((D // 2, F), I32),
        pltpu.VMEM((F // 2, D), I32),
        pltpu.VMEM((S + BR, D), F32),
        pltpu.VMEM((S + BR, D), F32),
        pltpu.VMEM((D // 128, S + 4 * PAD + BR, 128), F32),
        pltpu.VMEM((S + BR, D), BF),
        pltpu.VMEM((NP, RING, PW), F32),
        pltpu.VMEM((NP, RING, PW), F32),
        pltpu.VMEM((NP, RING, PW), F32),
        pltpu.VMEM((LA, D), F32),
        pltpu.SemaphoreType.DMA((1,)),
        pltpu.SemaphoreType.DMA((5, NP)),
        pltpu.SemaphoreType.DMA((4,)),
        pltpu.SemaphoreType.DMA((1,)),
    ]
    out = pl.pallas_call(
        _kernel,
        out_shape=jax.ShapeDtypeStruct((S, D), BF),
        in_specs=[any_spec] * 10,
        out_specs=any_spec,
        scratch_shapes=scratch,
        compiler_params=pltpu.CompilerParams(vmem_limit_bytes=126 * 1024 * 1024,
                                             disable_bounds_checks=NO_BOUNDS_CHECKS),
    )(x, mem0, wqt, wkt, wvt, wo, B_w1, B_w2, B_w3, B_w4)
    return out.reshape(1, S, D)


def pallas_interleave_layers__memory_aug_recurrent_mem_tr__mixer_s_mlp__prompt_kernel(
    A_x, A_mem0, A_Wq, A_Wk, A_Wv, A_Wo, A_seg_len, B_x, B_w1, B_w2, B_w3, B_w4,
):
    del B_x
    if isinstance(A_seg_len, int):
        assert A_seg_len == SEG
    assert A_x.shape == (1, S, D)
    return _impl(A_x, A_mem0, A_Wq, A_Wk, A_Wv, A_Wo, B_w1, B_w2, B_w3, B_w4)
```

```python
import contextlib

import jax
import jax.numpy as jnp
from jax import lax
import jax.experimental.pallas as pl
import jax.experimental.pallas.tpu as pltpu

BF = jnp.bfloat16
F32 = jnp.float32
I32 = jnp.int32

S, D, H, E, M, SEG, F = 2048, 640, 32, 192, 8, 32, 1536
L = M + SEG
NSEG = S // SEG
NP = H // 2
PW = 2 * E
SCALE = float(E ** -0.5)
EPS = 1e-5
TK = 24
LA = S - NSEG * TK
RING = LA + SEG
PAD = 8
GROUP = D // 4
XB = 128
NXH = LA // XB
NSL = 4
NBW, BW0 = 8, 6
UNROLL = 2
PRE_UNROLL = 4

LAGS = (1, 3, 5)
SLOT_ORDER = ('lv', 'v', 'out', 'lqk', 'q', 'k', 'qk', 'pv')
END = 99
HOOKS = ((1, 2, 6, 15, END), (1, 5, 11, 15, 18))
PROFILE = False


def _scope(name):
    return jax.named_scope(name) if PROFILE else contextlib.nullcontext()


def _ln(x):
    m = jnp.mean(x, axis=-1, keepdims=True)
    c = x - m
    v = jnp.mean(c * c, axis=-1, keepdims=True)
    return c * lax.rsqrt(v + EPS)


def _gelu(x):
    k = 0.7978845608028654
    return 0.5 * x * (1.0 + jnp.tanh(k * (x + 0.044715 * (x * x * x))))


def _dot(a, w):
    return jnp.dot(a, pltpu.bitcast(w, BF), preferred_element_type=F32)


def _a_step(h, rd, wr, weights, rings, hooks):
    wq, wk, wv, wo = weights
    lane = lax.broadcasted_iota(I32, (L, 128), 1)
    lo = lane < 64
    col = lax.broadcasted_iota(I32, (L, 2 * L), 1)
    row = lax.broadcasted_iota(I32, (L, 2 * L), 0)
    first = col < L
    key = jnp.where(first, col, col - L)
    allowed = (row < M) | (row >= key)
    zt = jnp.zeros((L, 128), F32)
    vals = ({}, {}, {})
    probs, outs, acc = {}, {}, [None]

    def blockdiag(t):
        t0, t1, t2 = t[:, 0:128], t[:, 128:256], t[:, 256:384]
        top = jnp.concatenate([t0, jnp.where(lo, t1, 0.0), zt], axis=1)
        bot = jnp.concatenate([zt, jnp.where(lo, 0.0, t1), t2], axis=1)
        return jnp.concatenate([top, bot], axis=0).astype(BF)

    def project(i):
        def fn(p):
            y = _dot(h, (wq, wk, wv)[i][p])
            for n, r in enumerate(wr):
                rings[i][p, pl.ds(r, 8), :] = y[M + 8 * n:M + 8 * n + 8, :]
            vals[i][p] = y[:M, :]
        return fn

    def gather(i, p):
        return jnp.concatenate([vals[i][p], rings[i][p, pl.ds(rd, SEG), :]], axis=0)

    def load_qk(p):
        vals[0][p] = gather(0, p)
        vals[1][p] = blockdiag(gather(1, p))

    def load_v(p):
        vals[2][p] = blockdiag(gather(2, p))

    def qk(p):
        s = lax.dot_general(vals[0].pop(p), vals[1].pop(p), (((1,), (1,)), ((), ())),
                            preferred_element_type=F32)
        s = jnp.where(allowed, s * SCALE, -1e9)
        m1 = jnp.max(jnp.where(first, s, -jnp.inf), axis=1, keepdims=True)
        m2 = jnp.max(jnp.where(first, -jnp.inf, s), axis=1, keepdims=True)
        e = jnp.exp(s - jnp.where(first, m1, m2))
        l1 = jnp.sum(jnp.where(first, e, 0.0), axis=1, keepdims=True)
        l2 = jnp.sum(jnp.where(first, 0.0, e), axis=1, keepdims=True)
        probs[p] = e * pl.reciprocal(jnp.where(first, l1, l2), approx=False)

    def pv(p):
        outs[p] = jnp.dot(probs.pop(p), vals[2].pop(p), preferred_element_type=F32)

    def out(p):
        y = _dot(outs.pop(p), wo[p])
        acc[0] = y if acc[0] is None else acc[0] + y

    la, lb, lc = LAGS
    ops = dict(q=(project(0), 0), k=(project(1), 0), v=(project(2), 0), lqk=(load_qk, la),
               lv=(load_v, lb), qk=(qk, la), pv=(pv, lb), out=(out, lc))
    for t in list(range(NP + lc)) + [END]:
        for fn in hooks.get(t, ()):
            fn()
        for name in SLOT_ORDER:
            fn, lag = ops[name]
            if 0 <= t - lag < NP:
                fn(t - lag)
    return acc[0]


def _shift_gather(hbuf, r0, rows):
    lane = lax.broadcasted_iota(I32, (rows, 128), 1)
    shifts = (-1, 1, -2, 2)
    tiles = []
    for t in range(D // 128):
        g_lo = (t * 128) // GROUP
        g_hi = (t * 128 + 127) // GROUP
        a = hbuf[t, pl.ds(r0 + shifts[g_lo], rows), :]
        if g_hi != g_lo:
            b = hbuf[t, pl.ds(r0 + shifts[g_hi], rows), :]
            a = jnp.where(lane < (g_hi * GROUP - t * 128), a, b)
        tiles.append(a)
    return jnp.concatenate(tiles, axis=1)


def _kernel(x_hbm, mem_hbm, wq_hbm, wk_hbm, wv_hbm, wo_hbm, w1_hbm, w2_hbm, w3_hbm, w4_hbm,
            o_hbm,
            xb, memb, sq, sk, sv, so, s1, s2, s3, s4,
            wq, wk, wv, wo, w1, w2, w3, w4,
            xres, xn, xa, hbuf, ob, rq, rk, rv, sem_m, sem_w, sem_b, sem_o):
    b_weights = ((w1_hbm, s1, w1), (w2_hbm, s2, w2), (w3_hbm, s3, w3), (w4_hbm, s4, w4))

    def mem_copy():
        return pltpu.make_async_copy(mem_hbm, memb, sem_m.at[0])

    def w_copy(i, p):
        src, dst = ((wq_hbm, sq), (wk_hbm, sk), (wv_hbm, sv), (wo_hbm, so))[i]
        return pltpu.make_async_copy(src.at[pl.ds(pl.multiple_of(p * PW, PW), PW), :],
                                     dst.at[lax.rem(p, NSL)], sem_w.at[i, p])

    def xblk_copy(b):
        xs = pl.ds(pl.multiple_of(b * XB, XB), XB)
        return pltpu.make_async_copy(x_hbm.at[xs, :], xb.at[xs, :], sem_w.at[4, b])

    def b_copies(k):
        cps = []
        for i, (src, dst, _) in enumerate(b_weights):
            n = src.shape[0] // NBW
            sl = pl.ds(pl.multiple_of(k * n, n), n)
            cps.append(pltpu.make_async_copy(src.at[sl, :], dst.at[sl, :], sem_b.at[i]))
        return cps

    def group(p, action, part=None):
        act = (lambda cp: cp.start()) if action == 'start' else (lambda cp: cp.wait())
        if part in (None, 0):
            @pl.when(p < NP)
            def _():
                act(w_copy(2, p))
        if part in (None, 1):
            @pl.when(p < NP)
            def _():
                act(w_copy(3, p))

            @pl.when(p + 1 < NP)
            def _():
                act(w_copy(0, p + 1))
                act(w_copy(1, p + 1))

            @pl.when(p + NXH < S // XB)
            def _():
                act(xblk_copy(p + NXH))

    def init_rows(x0, ln_dst):
        x = xb[pl.ds(x0, XB), :].astype(F32)
        xres[pl.ds(x0, XB), :] = x
        ln_dst[pl.ds(x0, XB), :] = _ln(x)

    def relayout(i, p):
        src, dst = ((sq, wq), (sk, wk), (sv, wv))[i]
        dst[p] = pltpu.bitcast(src[lax.rem(p, NSL)].T, I32)

    def pack_wo(p):
        wo[p] = pltpu.bitcast(so[lax.rem(p, NSL)], I32)

    def project_ahead(i, p, src):
        w, ring = ((wq, rq), (wk, rk), (wv, rv))[i]
        for c in range(LA // 128):
            ring[p, c * 128:(c + 1) * 128, :] = _dot(src[c * 128:(c + 1) * 128, :], w[p])

    w_copy(0, 0).start()
    for b in range(NXH):
        xblk_copy(b).start()
    mem_copy().start()

    hbuf[:, pl.ds(0, PAD), :] = jnp.zeros((D // 128, PAD, 128), F32)
    hbuf[:, pl.ds(PAD + S, 3 * PAD + SEG), :] = jnp.zeros((D // 128, 3 * PAD + SEG, 128), F32)
    xres[pl.ds(S, SEG), :] = jnp.zeros((SEG, D), F32)
    xn[pl.ds(S, SEG), :] = jnp.zeros((SEG, D), F32)

    with _scope('head'):
        xblk_copy(0).wait()
        w_copy(1, 0).start()
        group(0, 'start', 0)
        for b in range(1, NXH):
            xblk_copy(b).wait()
        w_copy(0, 0).wait()
        mem_copy().wait()
        group(0, 'start', 1)
        group(1, 'start', 0)
        for b in range(NXH):
            init_rows(b * XB, xa)
        relayout(0, 0)
        project_ahead(0, 0, xa)
        w_copy(1, 0).wait()
        relayout(1, 0)
        group(1, 'start', 1)

    def prep_block(p, carry):
        group(p, 'wait', 0)
        group(p + 2, 'start')

        @pl.when((p >= BW0) & (p < BW0 + NBW))
        def _():
            for cp in b_copies(p - BW0):
                cp.start()
        relayout(2, p)
        project_ahead(1, p, xa)
        group(p, 'wait', 1)
        relayout(0, p + 1)
        project_ahead(2, p, xa)
        pack_wo(p)
        relayout(1, p + 1)
        init_rows(pl.multiple_of(jnp.minimum(p + NXH, S // XB - 1) * XB, XB), xn)
        project_ahead(0, p + 1, xa)
        return carry

    with _scope('prep'):
        lax.fori_loop(0, NP - 1, prep_block, 0)
        group(NP - 1, 'wait')
        for i, (src, dst, _) in enumerate(b_weights):
            pltpu.make_async_copy(src, dst, sem_b.at[i]).wait()
        relayout(2, NP - 1)
        for _, src, dst in b_weights:
            dst[...] = pltpu.bitcast(src[...], I32)
        project_ahead(1, NP - 1, xa)
        project_ahead(2, NP - 1, xa)
        pack_wo(NP - 1)

    def b_rows(jb):
        valid = jb >= 0
        blk = lax.rem(jnp.maximum(jb, 0), NSEG)
        r0 = pl.multiple_of(jnp.where(valid, blk * SEG, S), SEG)
        h0 = pl.multiple_of(jnp.where(valid, blk * SEG + PAD, S + 3 * PAD), PAD)
        return r0, h0

    def b1_stages(jb):
        r0, h0 = b_rows(jb)
        st = {}

        def s_ln():
            xin = _ln(xres[pl.ds(r0, SEG), :])
            xn[pl.ds(r0, SEG), :] = xin
            st['t'] = _ln(xin)

        def s_w1():
            hh = _gelu(_dot(st.pop('t'), w1[...]))
            for t in range(D // 128):
                hbuf[t, pl.ds(h0, SEG), :] = hh[:, t * 128:(t + 1) * 128]
        return [s_ln, s_w1]

    def b2_stages(jb, rows=SEG):
        r0, h0 = b_rows(jb)
        st = {}

        def s_w2():
            x1 = xn[pl.ds(r0, rows), :] + _dot(_shift_gather(hbuf, h0, rows), w2[...])
            st['x1'] = x1
            st['u'] = _ln(x1)

        def s_w3():
            st['g'] = _gelu(_dot(st.pop('u'), w3[...]))

        def s_w4():
            xo = xres[pl.ds(r0, rows), :] + (st.pop('x1') + _dot(st.pop('g'), w4[...]))
            xres[pl.ds(r0, rows), :] = xo
            xn[pl.ds(r0, rows), :] = _ln(xo)
            ob[pl.ds(r0, rows), :] = xo.astype(BF)
        return [s_w2, s_w3, s_w4]

    def out_copy(blk, nblk):
        sl = pl.ds(pl.multiple_of(blk * SEG, SEG), SEG * nblk)
        return pltpu.make_async_copy(ob.at[sl, :], o_hbm.at[sl, :], sem_o.at[0])

    def step(j, mem, tok, hook_slots):
        hooks = {}
        for t, fn in zip(hook_slots, b1_stages(j - 1) + b2_stages(j - 2)):
            hooks.setdefault(t, []).append(fn)
        s = lax.rem(j, NSEG)
        mem = jnp.where(s == 0, memb[...].astype(F32), mem)
        r0 = pl.multiple_of(s * SEG, SEG)
        n0 = LA + s * TK
        rd = pl.multiple_of(lax.rem(r0, RING), SEG)
        wr = [pl.multiple_of(lax.rem(n0 + 8 * i, RING), 8) for i in range(TK // 8)]
        o = _a_step(jnp.concatenate([mem, tok], axis=0), rd, wr,
                    (wq, wk, wv, wo), (rq, rk, rv), hooks)
        xres[pl.ds(r0, SEG), :] = xres[pl.ds(r0, SEG), :] + o[M:, :]
        return o[:M, :]

    def iteration(jj, mem):
        j0 = jj * UNROLL

        @pl.when(j0 == NSEG)
        def _():
            def body(p, c):
                for i in range(3):
                    project_ahead(i, p, xn)
                return c
            lax.fori_loop(0, NP, body, 0, unroll=PRE_UNROLL)

        toks = [xn[pl.ds(pl.multiple_of(LA + lax.rem(j0 + u, NSEG) * TK, 8), TK), :]
                for u in range(UNROLL)]
        for u in range(UNROLL):
            mem = step(j0 + u, mem, toks[u], HOOKS[u])

        @pl.when(j0 - 2 >= NSEG)
        def _():
            out_copy(j0 - 2 - NSEG, UNROLL).start()
        return mem

    with _scope('main'):
        lax.fori_loop(0, 2 * NSEG // UNROLL, iteration, memb[...].astype(F32))

    with _scope('epilogue'):
        last = 2 * NSEG - 1
        for fn in b1_stages(last) + b2_stages(last - 1, 2 * SEG):
            fn()
        out_copy(NSEG - 2, 2).start()
    pltpu.make_async_copy(ob.at[pl.ds(0, S), :], o_hbm, sem_o.at[0]).wait()


@jax.jit
def _impl(A_x, A_mem0, A_Wq, A_Wk, A_Wv, A_Wo, B_w1, B_w2, B_w3, B_w4):
    x = A_x.reshape(S, D)
    mem0 = A_mem0.reshape(M, D)
    wqt, wkt, wvt = (jnp.transpose(w, (1, 2, 0)).reshape(H * E, D) for w in (A_Wq, A_Wk, A_Wv))
    wo = A_Wo.reshape(H * E, D)
    any_spec = pl.BlockSpec(memory_space=pl.ANY)
    scratch = (
        [pltpu.VMEM((S, D), BF), pltpu.VMEM((M, D), BF)]
        + [pltpu.VMEM((NSL, PW, D), BF)] * 4
        + [pltpu.VMEM(shape, BF) for shape in ((D, D), (D, D), (D, F), (F, D))]
        + [pltpu.VMEM((NP, D // 2, PW), I32)] * 3
        + [pltpu.VMEM((NP, PW // 2, D), I32)]
        + [pltpu.VMEM((r // 2, c), I32) for r, c in ((D, D), (D, D), (D, F), (F, D))]
        + [pltpu.VMEM((S + SEG, D), F32)] * 2
        + [pltpu.VMEM((LA, D), F32)]
        + [pltpu.VMEM((D // 128, S + 4 * PAD + SEG, 128), F32)]
        + [pltpu.VMEM((S + SEG, D), BF)]
        + [pltpu.VMEM((NP, RING, PW), F32)] * 3
        + [pltpu.SemaphoreType.DMA((1,)), pltpu.SemaphoreType.DMA((5, NP)),
           pltpu.SemaphoreType.DMA((4,)), pltpu.SemaphoreType.DMA((1,))])
    out = pl.pallas_call(
        _kernel,
        out_shape=jax.ShapeDtypeStruct((S, D), BF),
        in_specs=[any_spec] * 10,
        out_specs=any_spec,
        scratch_shapes=scratch,
        compiler_params=pltpu.CompilerParams(vmem_limit_bytes=126 * 1024 * 1024,
                                             disable_bounds_checks=True),
    )(x, mem0, wqt, wkt, wvt, wo, B_w1, B_w2, B_w3, B_w4)
    return out.reshape(1, S, D)


def pallas_interleave_layers__memory_aug_recurrent_mem_tr__mixer_s_mlp__prompt_kernel(
    A_x, A_mem0, A_Wq, A_Wk, A_Wv, A_Wo, A_seg_len, B_x, B_w1, B_w2, B_w3, B_w4,
):
    del B_x
    if isinstance(A_seg_len, int):
        assert A_seg_len == SEG
    assert A_x.shape == (1, S, D)
    return _impl(A_x, A_mem0, A_Wq, A_Wk, A_Wv, A_Wo, B_w1, B_w2, B_w3, B_w4)
```

```python
import contextlib

import jax
import jax.numpy as jnp
from jax import lax
import jax.experimental.pallas as pl
import jax.experimental.pallas.tpu as pltpu

BF = jnp.bfloat16
F32 = jnp.float32
I32 = jnp.int32

S, D, H, E, M, SEG, F = 2048, 640, 32, 192, 8, 32, 1536
L = M + SEG
NSEG = S // SEG
NP = H // 2
PW = 2 * E
SCALE = float(E ** -0.5)
EPS = 1e-5
TK = 24
LA = S - NSEG * TK
RING = LA + SEG
PAD = 8
GROUP = D // 4
XB = 128
NXH = LA // XB
NSL = 4
NBW, BW0 = 8, 6
UNROLL = 2
PRE_UNROLL = 4

LAGS = (1, 3, 5)
SLOT_ORDER = ('lv', 'v', 'out', 'lqk', 'q', 'k', 'qk', 'pv')
END = 99
HOOKS = ((1, 2, 6, 15, END), (1, 5, 11, 15, 18))
PROFILE = False


def _scope(name):
    return jax.named_scope(name) if PROFILE else contextlib.nullcontext()


def _ln(x):
    m = jnp.mean(x, axis=-1, keepdims=True)
    c = x - m
    v = jnp.mean(c * c, axis=-1, keepdims=True)
    return c * lax.rsqrt(v + EPS)


def _gelu(x):
    k = 0.7978845608028654
    return 0.5 * x * (1.0 + jnp.tanh(k * (x + 0.044715 * (x * x * x))))


def _dot(a, w):
    return jnp.dot(a, pltpu.bitcast(w, BF), preferred_element_type=F32)


def _a_step(h, rd, wr, weights, rings, hooks):
    wq, wk, wv, wo = weights
    lane = lax.broadcasted_iota(I32, (L, 128), 1)
    lo = lane < 64
    col = lax.broadcasted_iota(I32, (L, 2 * L), 1)
    row = lax.broadcasted_iota(I32, (L, 2 * L), 0)
    first = col < L
    key = jnp.where(first, col, col - L)
    allowed = (row < M) | (row >= key)
    zt = jnp.zeros((L, 128), F32)
    vals = ({}, {}, {})
    probs, outs, acc = {}, {}, [None]

    def blockdiag(t):
        t0, t1, t2 = t[:, 0:128], t[:, 128:256], t[:, 256:384]
        top = jnp.concatenate([t0, jnp.where(lo, t1, 0.0), zt], axis=1)
        bot = jnp.concatenate([zt, jnp.where(lo, 0.0, t1), t2], axis=1)
        return jnp.concatenate([top, bot], axis=0).astype(BF)

    def project(i):
        def fn(p):
            y = _dot(h, (wq, wk, wv)[i][p])
            for n, r in enumerate(wr):
                rings[i][p, pl.ds(r, 8), :] = y[M + 8 * n:M + 8 * n + 8, :]
            vals[i][p] = y[:M, :]
        return fn

    def gather(i, p):
        return jnp.concatenate([vals[i][p], rings[i][p, pl.ds(rd, SEG), :]], axis=0)

    def load_qk(p):
        vals[0][p] = gather(0, p)
        vals[1][p] = blockdiag(gather(1, p))

    def load_v(p):
        vals[2][p] = blockdiag(gather(2, p))

    def qk(p):
        s = lax.dot_general(vals[0].pop(p), vals[1].pop(p), (((1,), (1,)), ((), ())),
                            preferred_element_type=F32)
        s = jnp.where(allowed, s * SCALE, -1e9)
        m1 = jnp.max(jnp.where(first, s, -jnp.inf), axis=1, keepdims=True)
        m2 = jnp.max(jnp.where(first, -jnp.inf, s), axis=1, keepdims=True)
        e = jnp.exp(s - jnp.where(first, m1, m2))
        l1 = jnp.sum(jnp.where(first, e, 0.0), axis=1, keepdims=True)
        l2 = jnp.sum(jnp.where(first, 0.0, e), axis=1, keepdims=True)
        probs[p] = e * pl.reciprocal(jnp.where(first, l1, l2), approx=False)

    def pv(p):
        outs[p] = jnp.dot(probs.pop(p), vals[2].pop(p), preferred_element_type=F32)

    def out(p):
        y = _dot(outs.pop(p), wo[p])
        acc[0] = y if acc[0] is None else acc[0] + y

    la, lb, lc = LAGS
    ops = dict(q=(project(0), 0), k=(project(1), 0), v=(project(2), 0), lqk=(load_qk, la),
               lv=(load_v, lb), qk=(qk, la), pv=(pv, lb), out=(out, lc))
    for t in list(range(NP + lc)) + [END]:
        for fn in hooks.get(t, ()):
            fn()
        for name in SLOT_ORDER:
            fn, lag = ops[name]
            if 0 <= t - lag < NP:
                fn(t - lag)
    return acc[0]


def _shift_gather(hbuf, r0, rows):
    lane = lax.broadcasted_iota(I32, (rows, 128), 1)
    shifts = (-1, 1, -2, 2)
    tiles = []
    for t in range(D // 128):
        g_lo = (t * 128) // GROUP
        g_hi = (t * 128 + 127) // GROUP
        a = hbuf[t, pl.ds(r0 + shifts[g_lo], rows), :]
        if g_hi != g_lo:
            b = hbuf[t, pl.ds(r0 + shifts[g_hi], rows), :]
            a = jnp.where(lane < (g_hi * GROUP - t * 128), a, b)
        tiles.append(a)
    return jnp.concatenate(tiles, axis=1)


def _kernel(x_hbm, mem_hbm, wq_hbm, wk_hbm, wv_hbm, wo_hbm, w1_hbm, w2_hbm, w3_hbm, w4_hbm,
            o_hbm,
            xb, memb, sq, sk, sv, so, s1, s2, s3, s4,
            wq, wk, wv, wo, w1, w2, w3, w4,
            xres, xn, xa, hbuf, ob, rq, rk, rv, sem_m, sem_w, sem_b, sem_o):
    b_weights = ((w1_hbm, s1, w1), (w2_hbm, s2, w2), (w3_hbm, s3, w3), (w4_hbm, s4, w4))

    def mem_copy():
        return pltpu.make_async_copy(mem_hbm, memb, sem_m.at[0])

    def w_copy(i, p):
        src, dst = ((wq_hbm, sq), (wk_hbm, sk), (wv_hbm, sv), (wo_hbm, so))[i]
        return pltpu.make_async_copy(src.at[pl.ds(pl.multiple_of(p * PW, PW), PW), :],
                                     dst.at[lax.rem(p, NSL)], sem_w.at[i, p])

    def xblk_copy(b):
        xs = pl.ds(pl.multiple_of(b * XB, XB), XB)
        return pltpu.make_async_copy(x_hbm.at[xs, :], xb.at[xs, :], sem_w.at[4, b])

    def b_copies(k):
        cps = []
        for i, (src, dst, _) in enumerate(b_weights):
            n = src.shape[0] // NBW
            sl = pl.ds(pl.multiple_of(k * n, n), n)
            cps.append(pltpu.make_async_copy(src.at[sl, :], dst.at[sl, :], sem_b.at[i]))
        return cps

    def group(p, action, part=None):
        act = (lambda cp: cp.start()) if action == 'start' else (lambda cp: cp.wait())
        if part in (None, 0):
            @pl.when(p < NP)
            def _():
                act(w_copy(2, p))
        if part in (None, 1):
            @pl.when(p < NP)
            def _():
                act(w_copy(3, p))

            @pl.when(p + 1 < NP)
            def _():
                act(w_copy(0, p + 1))
                act(w_copy(1, p + 1))

            @pl.when(p + NXH < S // XB)
            def _():
                act(xblk_copy(p + NXH))

    def init_rows(x0, ln_dst):
        x = xb[pl.ds(x0, XB), :].astype(F32)
        xres[pl.ds(x0, XB), :] = x
        ln_dst[pl.ds(x0, XB), :] = _ln(x)

    def relayout(i, p):
        src, dst = ((sq, wq), (sk, wk), (sv, wv))[i]
        dst[p] = pltpu.bitcast(src[lax.rem(p, NSL)].T, I32)

    def pack_wo(p):
        wo[p] = pltpu.bitcast(so[lax.rem(p, NSL)], I32)

    def project_ahead(i, p, src):
        w, ring = ((wq, rq), (wk, rk), (wv, rv))[i]
        for c in range(LA // 128):
            ring[p, c * 128:(c + 1) * 128, :] = _dot(src[c * 128:(c + 1) * 128, :], w[p])

    w_copy(0, 0).start()
    for b in range(NXH):
        xblk_copy(b).start()
    mem_copy().start()

    hbuf[:, pl.ds(0, PAD), :] = jnp.zeros((D // 128, PAD, 128), F32)
    hbuf[:, pl.ds(PAD + S, 3 * PAD + SEG), :] = jnp.zeros((D // 128, 3 * PAD + SEG, 128), F32)
    xres[pl.ds(S, SEG), :] = jnp.zeros((SEG, D), F32)
    xn[pl.ds(S, SEG), :] = jnp.zeros((SEG, D), F32)

    with _scope('head'):
        xblk_copy(0).wait()
        w_copy(1, 0).start()
        group(0, 'start', 0)
        for b in range(1, NXH):
            xblk_copy(b).wait()
        w_copy(0, 0).wait()
        mem_copy().wait()
        group(0, 'start', 1)
        group(1, 'start', 0)
        for b in range(NXH):
            init_rows(b * XB, xa)
        relayout(0, 0)
        project_ahead(0, 0, xa)
        w_copy(1, 0).wait()
        relayout(1, 0)
        group(1, 'start', 1)

    def prep_block(p, carry):
        group(p, 'wait', 0)
        group(p + 2, 'start')

        @pl.when((p >= BW0) & (p < BW0 + NBW))
        def _():
            for cp in b_copies(p - BW0):
                cp.start()
        relayout(2, p)
        project_ahead(1, p, xa)
        group(p, 'wait', 1)
        relayout(0, p + 1)
        project_ahead(2, p, xa)
        pack_wo(p)
        relayout(1, p + 1)
        init_rows(pl.multiple_of(jnp.minimum(p + NXH, S // XB - 1) * XB, XB), xn)
        project_ahead(0, p + 1, xa)
        return carry

    with _scope('prep'):
        lax.fori_loop(0, NP - 1, prep_block, 0)
        group(NP - 1, 'wait')
        for i, (src, dst, _) in enumerate(b_weights):
            pltpu.make_async_copy(src, dst, sem_b.at[i]).wait()
        relayout(2, NP - 1)
        for _, src, dst in b_weights:
            dst[...] = pltpu.bitcast(src[...], I32)
        project_ahead(1, NP - 1, xa)
        project_ahead(2, NP - 1, xa)
        pack_wo(NP - 1)

    def b_rows(jb):
        valid = jb >= 0
        blk = lax.rem(jnp.maximum(jb, 0), NSEG)
        r0 = pl.multiple_of(jnp.where(valid, blk * SEG, S), SEG)
        h0 = pl.multiple_of(jnp.where(valid, blk * SEG + PAD, S + 3 * PAD), PAD)
        return r0, h0

    def b1_stages(jb):
        r0, h0 = b_rows(jb)
        st = {}

        def s_ln():
            xin = _ln(xres[pl.ds(r0, SEG), :])
            xn[pl.ds(r0, SEG), :] = xin
            st['t'] = _ln(xin)

        def s_w1():
            hh = _gelu(_dot(st.pop('t'), w1[...]))
            for t in range(D // 128):
                hbuf[t, pl.ds(h0, SEG), :] = hh[:, t * 128:(t + 1) * 128]
        return [s_ln, s_w1]

    def b2_stages(jb, rows=SEG):
        r0, h0 = b_rows(jb)
        st = {}

        def s_w2():
            x1 = xn[pl.ds(r0, rows), :] + _dot(_shift_gather(hbuf, h0, rows), w2[...])
            st['x1'] = x1
            st['u'] = _ln(x1)

        def s_w3():
            st['g'] = _gelu(_dot(st.pop('u'), w3[...]))

        def s_w4():
            xo = xres[pl.ds(r0, rows), :] + (st.pop('x1') + _dot(st.pop('g'), w4[...]))
            xres[pl.ds(r0, rows), :] = xo
            xn[pl.ds(r0, rows), :] = _ln(xo)
            ob[pl.ds(r0, rows), :] = xo.astype(BF)
        return [s_w2, s_w3, s_w4]

    def out_copy(blk, nblk):
        sl = pl.ds(pl.multiple_of(blk * SEG, SEG), SEG * nblk)
        return pltpu.make_async_copy(ob.at[sl, :], o_hbm.at[sl, :], sem_o.at[0])

    def step(j, mem, tok, hook_slots):
        hooks = {}
        for t, fn in zip(hook_slots, b1_stages(j - 1) + b2_stages(j - 2)):
            hooks.setdefault(t, []).append(fn)
        s = lax.rem(j, NSEG)
        mem = jnp.where(s == 0, memb[...].astype(F32), mem)
        r0 = pl.multiple_of(s * SEG, SEG)
        n0 = LA + s * TK
        rd = pl.multiple_of(lax.rem(r0, RING), SEG)
        wr = [pl.multiple_of(lax.rem(n0 + 8 * i, RING), 8) for i in range(TK // 8)]
        o = _a_step(jnp.concatenate([mem, tok], axis=0), rd, wr,
                    (wq, wk, wv, wo), (rq, rk, rv), hooks)
        xres[pl.ds(r0, SEG), :] = xres[pl.ds(r0, SEG), :] + o[M:, :]
        return o[:M, :]

    def iteration(jj, mem):
        j0 = jj * UNROLL

        @pl.when(j0 == NSEG)
        def _():
            def body(p, c):
                for i in range(3):
                    project_ahead(i, p, xn)
                return c
            lax.fori_loop(0, NP, body, 0, unroll=PRE_UNROLL)

        toks = [xn[pl.ds(pl.multiple_of(LA + lax.rem(j0 + u, NSEG) * TK, 8), TK), :]
                for u in range(UNROLL)]
        for u in range(UNROLL):
            mem = step(j0 + u, mem, toks[u], HOOKS[u])

        @pl.when(j0 - UNROLL >= NSEG)
        def _():
            out_copy(j0 - UNROLL - NSEG, UNROLL).start()
        return mem

    with _scope('main'):
        lax.fori_loop(0, 2 * NSEG // UNROLL, iteration, memb[...].astype(F32))

    with _scope('epilogue'):
        last = 2 * NSEG - 1
        if UNROLL > 2:
            out_copy(NSEG - UNROLL, UNROLL - 2).start()
        for fn in b1_stages(last) + b2_stages(last - 1, 2 * SEG):
            fn()
        out_copy(NSEG - 2, 2).start()
    pltpu.make_async_copy(ob.at[pl.ds(0, S), :], o_hbm, sem_o.at[0]).wait()


@jax.jit
def _impl(A_x, A_mem0, A_Wq, A_Wk, A_Wv, A_Wo, B_w1, B_w2, B_w3, B_w4):
    x = A_x.reshape(S, D)
    mem0 = A_mem0.reshape(M, D)
    wqt, wkt, wvt = (jnp.transpose(w, (1, 2, 0)).reshape(H * E, D) for w in (A_Wq, A_Wk, A_Wv))
    wo = A_Wo.reshape(H * E, D)
    any_spec = pl.BlockSpec(memory_space=pl.ANY)
    scratch = (
        [pltpu.VMEM((S, D), BF), pltpu.VMEM((M, D), BF)]
        + [pltpu.VMEM((NSL, PW, D), BF)] * 4
        + [pltpu.VMEM(shape, BF) for shape in ((D, D), (D, D), (D, F), (F, D))]
        + [pltpu.VMEM((NP, D // 2, PW), I32)] * 3
        + [pltpu.VMEM((NP, PW // 2, D), I32)]
        + [pltpu.VMEM((r // 2, c), I32) for r, c in ((D, D), (D, D), (D, F), (F, D))]
        + [pltpu.VMEM((S + SEG, D), F32)] * 2
        + [pltpu.VMEM((LA, D), F32)]
        + [pltpu.VMEM((D // 128, S + 4 * PAD + SEG, 128), F32)]
        + [pltpu.VMEM((S + SEG, D), BF)]
        + [pltpu.VMEM((NP, RING, PW), F32)] * 3
        + [pltpu.SemaphoreType.DMA((1,)), pltpu.SemaphoreType.DMA((5, NP)),
           pltpu.SemaphoreType.DMA((4,)), pltpu.SemaphoreType.DMA((1,))])
    out = pl.pallas_call(
        _kernel,
        out_shape=jax.ShapeDtypeStruct((S, D), BF),
        in_specs=[any_spec] * 10,
        out_specs=any_spec,
        scratch_shapes=scratch,
        compiler_params=pltpu.CompilerParams(vmem_limit_bytes=126 * 1024 * 1024,
                                             disable_bounds_checks=True),
    )(x, mem0, wqt, wkt, wvt, wo, B_w1, B_w2, B_w3, B_w4)
    return out.reshape(1, S, D)


def pallas_interleave_layers__memory_aug_recurrent_mem_tr__mixer_s_mlp__prompt_kernel(
    A_x, A_mem0, A_Wq, A_Wk, A_Wv, A_Wo, A_seg_len, B_x, B_w1, B_w2, B_w3, B_w4,
):
    del B_x
    if isinstance(A_seg_len, int):
        assert A_seg_len == SEG
    assert A_x.shape == (1, S, D)
    return _impl(A_x, A_mem0, A_Wq, A_Wk, A_Wv, A_Wo, B_w1, B_w2, B_w3, B_w4)
```
